```python
import jax
import jax.numpy as jnp

def _softmax(x, axis=-1):
    return jax.nn.softmax(x, axis=axis)

def _gelu(x):
    return jax.nn.gelu(x, approximate=True)

def _silu(x):
    return jax.nn.silu(x)

def _sigmoid(x):
    return jax.nn.sigmoid(x)

def _layernorm(x, axis=-1, eps=1e-05):
    m = jnp.mean(x, axis=axis, keepdims=True)
    v = jnp.var(x, axis=axis, keepdims=True)
    return (x - m) / jnp.sqrt(v + eps)

def _scatter_add(tgt, idx, src, axis=0):
    return tgt.at[idx].add(src)

def _segment_sum(src, seg, n):
    return jax.ops.segment_sum(src, seg, n)

class _Rng:

    def __init__(self, key):
        self._k = key

    def _next(self):
        self._k, sub = jax.random.split(self._k)
        return sub

    def normal(self, shape):
        return jax.random.normal(self._next(), shape, dtype=jnp.bfloat16)

    def randint(self, lo, hi, shape):
        return jax.random.randint(self._next(), shape, lo, hi, dtype=jnp.int32)

    def uniform(self, shape, lo=0.0, hi=1.0):
        return jax.random.uniform(self._next(), shape, jnp.bfloat16, lo, hi)

    def permutation(self, n):
        return jax.random.permutation(self._next(), n)
kernel_name = 'adaLN_cond__sliding_local_dilated__glu_gated_swiglu__prompt'

def setup_inputs():
    _rng = _Rng(jax.random.key(int.from_bytes(__import__("os").urandom(4), "little")))
    _w = lambda a: (lambda t: t.astype(jnp.bfloat16) if jnp.issubdtype(t.dtype, jnp.floating) else t)(jnp.asarray(a))

    def _A_setup():
        B, S, D = (1, 2048, 1024)
        return {'x': _w((lambda *s: _rng.normal(s) * 0.05)(B, S, D)), 'wqkv': _w((lambda *s: _rng.normal(s) * 0.05)(D, 3 * D)), 'wo': _w((lambda *s: _rng.normal(s) * 0.05)(D, D))}
    _A_in = _A_setup()

    def _B_setup():
        B, S, D, F = (1, 2048, 1024, 3584)
        return {'x': _w((lambda *s: _rng.normal(s) * 0.05)(B, S, D)), 'w1': _w((lambda *s: _rng.normal(s) * 0.05)(D, F) * (2.0 / D) ** 0.5), 'w3': _w((lambda *s: _rng.normal(s) * 0.05)(D, F) * (2.0 / D) ** 0.5), 'w2': _w((lambda *s: _rng.normal(s) * 0.05)(F, D) * (2.0 / F) ** 0.5)}
    _B_in = _B_setup()
    return {'A_x': _A_in['x'], 'A_wqkv': _A_in['wqkv'], 'A_wo': _A_in['wo'], 'B_x': _B_in['x'], 'B_w1': _B_in['w1'], 'B_w3': _B_in['w3'], 'B_w2': _B_in['w2'], 'c': _w((lambda *s: _rng.normal(s) * 0.05)(1, 1024)), 'w_mod': _w((lambda *s: _rng.normal(s) * 0.05)(1024, 6 * 1024) * 1024 ** (-0.5))}

def reference(A_x, A_wqkv, A_wo, B_x, B_w1, B_w3, B_w2, c, w_mod):

    def _A_ref(x, wqkv, wo):
        B, S, D = x.shape
        H = 32
        Dh = D // H
        W, dil = (8, 2)
        qkv = (lambda x, *d: x.transpose(*d))((x @ wqkv).reshape(B, S, 3, H, Dh), 2, 0, 3, 1, 4)
        q, k, v = (qkv[0], qkv[1], qkv[2])
        scale = Dh ** (-0.5)
        pos = jnp.arange(S)
        off = jnp.arange(W) * dil
        idx = pos[:, None] - off[None, :]
        mask = idx >= 0
        idx_c = jnp.where(mask, idx, 0).reshape(-1)
        kg = k[:, :, idx_c, :].reshape(B, H, S, W, Dh)
        vg = v[:, :, idx_c, :].reshape(B, H, S, W, Dh)
        logits = jnp.einsum('bhsd,bhswd->bhsw', q, kg) * scale
        logits = jnp.where(mask[None, None, :, :], logits, -1000000000.0)
        attn = _softmax(logits, axis=-1)
        o = jnp.einsum('bhsw,bhswd->bhsd', attn, vg)
        return (lambda x, *d: x.transpose(*d))(o, 0, 2, 1, 3).reshape(B, S, D) @ wo

    def _B_ref(x, w1, w3, w2):
        gate = jnp.einsum('bsd,df->bsf', x, w1)
        up = jnp.einsum('bsd,df->bsf', x, w3)
        h = _silu(gate) * up
        out = jnp.einsum('bsf,fd->bsd', h, w2)
        return out
    x = A_x
    mod = (_silu(c) @ w_mod).reshape(c.shape[0], 6, 1, -1)
    sa, ca, ga, sb, cb, gb = (mod[:, 0].copy(), mod[:, 1].copy(), mod[:, 2].copy(), mod[:, 3].copy(), mod[:, 4].copy(), mod[:, 5].copy())
    h = _layernorm(x, axis=-1) * (1 + ca) + sa
    x = x + ga * _A_ref(h, A_wqkv, A_wo)
    h = _layernorm(x, axis=-1) * (1 + cb) + sb
    x = x + gb * _B_ref(h, B_w1, B_w3, B_w2)
    return x
```

```python
import functools
import jax
import jax.numpy as jnp
from jax import lax
from jax.experimental import pallas as pl
from jax.experimental.pallas import tpu as pltpu

S, D, F = 2048, 1024, 3584
NP = 8
NU = 4
TM = 256
LOG2E = 1.4426950408889634
QSCALE = (32 ** -0.5) * LOG2E
EPS = 1e-5
SPAD = 2064
WPAD = 1032


def zero_of(v):
    b = pltpu.bitcast(v, jnp.uint32)
    return (b >> 31) >> 1


def tie_lhs(h, ties):
    if not ties:
        return h
    K = h.shape[1]
    nk = K // 512 if K >= 512 else 1
    kw = 512 if K >= 512 else K
    rows = []
    for g in range(h.shape[0] // 16):
        blk = h[16 * g:16 * g + 16, :]
        if any((g, kh) in ties for kh in range(nk)):
            cols = []
            for kh in range(nk):
                a = blk[:, kh * kw:(kh + 1) * kw]
                if (g, kh) in ties:
                    a0 = pltpu.bitcast(pltpu.bitcast(a[:, :128], jnp.uint32) | ties[(g, kh)], jnp.bfloat16)
                    a = jnp.concatenate([a0, a[:, 128:]], axis=1)
                cols.append(a)
            blk = jnp.concatenate(cols, axis=1) if len(cols) > 1 else cols[0]
        rows.append(blk)
    return jnp.concatenate(rows, axis=0)


def layer_norm(x):
    mean = jnp.sum(x, axis=1, keepdims=True) * (1.0 / D)
    xc = x - mean
    var = jnp.sum(xc * xc, axis=1, keepdims=True) * (1.0 / D)
    return xc * lax.rsqrt(var + EPS)


def load_words_bf16(buf, p):
    parts = [pltpu.bitcast(buf.at[j].bitcast(jnp.uint32)[pl.ds(p, 128, stride=8), :], jnp.bfloat16)
             for j in range(8)]
    return jnp.concatenate(parts, axis=1)


def store_words(buf_u32, p, val_bf16):
    wd = pltpu.bitcast(val_bf16, jnp.uint32)
    for j in range(8):
        buf_u32[j, pl.ds(p, 128, stride=8), :] = wd[:, 128 * j:128 * (j + 1)]
    return wd


def qdot(h, WQKV, R, p, t, u, ties):
    h = tie_lhs(h, ties)
    col = t * D + 256 * u
    r = jnp.dot(h, WQKV[:, col:col + 256], preferred_element_type=jnp.float32)
    marker = r[0:8, 0:128]
    if t == 0:
        r = r * QSCALE
    wd = pltpu.bitcast(r.astype(jnp.bfloat16), jnp.uint32)
    off = 0 if t == 0 else 16
    for j in range(2):
        wt = wd[:, j * 128:(j + 1) * 128].T
        for hf in range(2):
            rho = 2 * p + hf
            val = pltpu.unpack_elementwise(wt, index=hf, packed_dtype=jnp.bfloat16, unpacked_dtype=jnp.float32)
            for hh in range(4):
                R[off + rho, pl.ds(4 * j + hh, 32, stride=8), :] = val[32 * hh:32 * hh + 32]
            if t > 0:
                sv = pltpu.roll(val, 1, 1)
                for hh in range(4):
                    R[rho, pl.ds(4 * j + hh, 32, stride=8), :] = sv[32 * hh:32 * hh + 32]
    return marker


def attend_steps(RQ, RK, RV, p):
    lane = lax.broadcasted_iota(jnp.int32, (8, 128), 1)
    markers = []
    Ps = []
    for hf in range(2):
        rho = 2 * p + hf
        q = RQ[rho].reshape(32, 8, 128)
        Ls = []
        for w in range(8):
            kap = rho - 2 * w
            kk = RK[16 + kap].reshape(32, 8, 128)
            L = jnp.sum(q * kk, axis=0)
            if w > 0:
                thr = jnp.where(kap < 0, 0, -1)
                L = jnp.where(lane <= thr, -1e9, L)
            Ls.append(L)
            markers.append(zero_of(L))
        m = functools.reduce(jnp.maximum, Ls)
        es = [jnp.exp2(L - m) for L in Ls]
        ssum = functools.reduce(jnp.add, es)
        inv = 1.0 / ssum
        Ps.append([e * inv for e in es])
        markers.append(zero_of(inv))
    words = []
    for dg in range(16):
        ws = []
        for d in range(2 * dg, 2 * dg + 2):
            os_ = []
            for hf in range(2):
                rho = 2 * p + hf
                o = None
                for w in range(8):
                    kap = rho - 2 * w
                    vv = RV[16 + kap, 8 * d:8 * d + 8, :]
                    tt = Ps[hf][w] * vv
                    o = tt if o is None else o + tt
                os_.append(o)
            ws.append(pltpu.pack_elementwise(os_, packed_dtype=jnp.bfloat16))
        words += ws
        markers.append(zero_of(ws[0] | ws[1]))
    return markers, words


def store_o(OS, p, words, throttle):
    if throttle is not None:
        words = [w | throttle for w in words]
    OS[p, 0:256, :] = jnp.concatenate(words, axis=0)


def out_dot(OS, p, WO, u, ties=None):
    parts = []
    for jj in range(2):
        rows = [OS[p, pl.ds(4 * jj + hh, 32, stride=8), :] for hh in range(4)]
        nat = jnp.concatenate(rows, axis=0)
        parts.append(pltpu.bitcast(nat.T, jnp.bfloat16))
    lhs = jnp.concatenate(parts, axis=1)
    lhs = tie_lhs(lhs, ties)
    return jnp.dot(lhs, WO[256 * u:256 * u + 256, :], preferred_element_type=jnp.float32)


def spread(markers, slots, lo, hi):
    ties = {}
    n = len(markers)
    for i, mk in enumerate(markers):
        t, kh, g = slots[lo + (i * (hi - lo)) // n]
        ties.setdefault(t, {})
        key = (g, kh)
        ties[t][key] = mk if key not in ties[t] else (ties[t][key] | mk)
    return ties


SLOTS_QKV = [(t, kh, g) for t in range(3) for kh in range(2) for g in range(16)]


def make_kernel(cfg):
    unroll_u = cfg.get('unroll_u', 1)

    def kernel(x_hbm, wqkv_hbm, wo_hbm, w1_hbm, w3_hbm, w2_hbm, c_ref, wmod_hbm, out_hbm,
               XB, HP, WQKV, RQ0, RK0, RV0, RQ1, RK1, RV1, OS0, OS1, WO, ACC, H2B, X1B,
               W1, W3, W2, WMOD, OUTB, MOD, sems):
        Rset = [(RQ0, RK0, RV0), (RQ1, RK1, RV1)]
        OSs = [OS0, OS1]
        sem_i = [0]

        def new_copy(src, dst):
            i = sem_i[0]
            sem_i[0] += 1
            return pltpu.make_async_copy(src, dst, sems.at[i])

        cp_x = [new_copy(x_hbm.at[0, :, pl.ds(128 * j, 128)], XB.at[j, pl.ds(0, S), :]) for j in range(8)]
        cp_mod = [new_copy(wmod_hbm.at[:, pl.ds(1024 * i, 1024)], WMOD.at[:, pl.ds(1024 * i, 1024)]) for i in range(6)]
        cp_qkv = [[new_copy(wqkv_hbm.at[:, pl.ds(t * D + 256 * u, 256)], WQKV.at[:, pl.ds(t * D + 256 * u, 256)])
                   for t in range(3)] for u in range(NU)]
        cp_wo = new_copy(wo_hbm, WO)
        cp_w1 = new_copy(w1_hbm, W1)
        cp_w3 = new_copy(w3_hbm, W3)
        cp_w2 = new_copy(w2_hbm, W2)


        for c_ in cp_x:
            c_.start()
        cp_mod[0].start()
        cp_mod[1].start()
        for c_ in cp_qkv[0]:
            c_.start()
        for c_ in cp_x:
            c_.wait()
        for p in range(NP):
            xp = load_words_bf16(XB, p).astype(jnp.float32)
            ACC[p] = layer_norm(xp)
        cv = c_ref[...].astype(jnp.float32)
        sc = (cv * jax.nn.sigmoid(cv)).astype(jnp.bfloat16)
        sc16 = jnp.broadcast_to(sc, (16, D))
        cp_mod[0].wait()
        cp_mod[1].wait()
        m01 = jnp.dot(sc16, WMOD[:, 0:2048], preferred_element_type=jnp.float32)
        sa = m01[0:8, 0:1024]
        a1 = 1.0 + m01[0:8, 1024:2048]
        for c_ in cp_qkv[0]:
            c_.wait()
        for c_ in cp_qkv[1]:
            c_.start()
        cp_wo.start()
        for i in range(2, 6):
            cp_mod[i].start()

        sa_t = jnp.tile(sa, (TM // 8, 1))
        a1_t = jnp.tile(a1, (TM // 8, 1))
        for p in range(NP):
            h = (ACC[p] * a1_t + sa_t).astype(jnp.bfloat16)
            HP[p] = h
            for t in range(3):
                qdot(h, WQKV, Rset[0][t], p, t, 0, None)

        for u in range(1, NU):
            for c_ in cp_qkv[u]:
                c_.wait()
            if u == 1:
                cp_wo.wait()
                cp_w1.start()
            if u == 2:
                cp_w3.start()
            if u == 3:
                cp_w2.start()
            if u + 1 < NU:
                for c_ in cp_qkv[u + 1]:
                    c_.start()
            Rw = Rset[u % 2]
            Rr = Rset[(u - 1) % 2]
            OS = OSs[(u - 1) % 2]
            with_out = u <= 2

            def body(p, _, u=u, Rw=Rw, Rr=Rr, OS=OS, with_out=with_out):
                markers, words = attend_steps(Rr[0], Rr[1], Rr[2], p)
                ties = spread(markers, SLOTS_QKV, 2, 82)
                h = HP[p]
                ms = [qdot(h, WQKV, Rw[t], p, t, u, ties.get(t)) for t in range(3)]
                store_o(OS, p, words, zero_of(ms[2]))
                if with_out:
                    res = out_dot(OS, p, WO, u - 1)
                    if u == 1:
                        ACC[p] = res
                    else:
                        ACC[p] += res
                return 0
            lax.fori_loop(0, NP, body, 0, unroll=unroll_u)

        for i in range(2, 6):
            cp_mod[i].wait()

        def body_t1(p, _):
            markers, words = attend_steps(RQ1, RK1, RV1, p)
            n = len(markers)
            slots = [(0, 0, g) for g in range(16)]
            ties = spread(markers, slots, 0, 16)
            res = out_dot(OS0, p, WO, 2, ties.get(0))
            store_o(OS1, p, words, zero_of(res[0:8, 0:128]))
            ACC[p] += res
            return 0
        lax.fori_loop(0, NP, body_t1, 0)

        m2 = jnp.dot(sc16, WMOD[:, 2048:6144], preferred_element_type=jnp.float32)
        ga = m2[0:8, 0:1024]
        sb = m2[0:8, 1024:2048]
        b1 = 1.0 + m2[0:8, 2048:3072]
        gb = m2[0:8, 3072:4096]
        MOD[...] = gb
        ga_t = jnp.tile(ga, (TM // 8, 1))
        sb_t = jnp.tile(sb, (TM // 8, 1))
        b1_t = jnp.tile(b1, (TM // 8, 1))

        for p in range(NP):
            res = out_dot(OS1, p, WO, 3)
            a = ACC[p] + res
            xp = load_words_bf16(XB, p).astype(jnp.float32)
            x1 = (xp + ga_t * a).astype(jnp.bfloat16)
            store_words(X1B, p, x1)
            h2 = (layer_norm(x1.astype(jnp.float32)) * b1_t + sb_t).astype(jnp.bfloat16)
            store_words(H2B, p, h2)

        cp_w1.wait()
        cp_w3.wait()
        cp_w2.wait()
        TN = 512

        def ffn_body(r, _):
            w0 = pl.multiple_of(r * 128, 128)
            h = jnp.concatenate([pltpu.bitcast(H2B[j, pl.ds(w0, 128), :], jnp.bfloat16) for j in range(8)], axis=1)
            acc = None
            for j in range(F // TN):
                g = jnp.dot(h, W1[:, j * TN:(j + 1) * TN], preferred_element_type=jnp.float32)
                up = jnp.dot(h, W3[:, j * TN:(j + 1) * TN], preferred_element_type=jnp.float32)
                a = (g * jax.nn.sigmoid(g) * up).astype(jnp.bfloat16)
                o = jnp.dot(a, W2[j * TN:(j + 1) * TN, :], preferred_element_type=jnp.float32)
                acc = o if acc is None else acc + o
            x1 = jnp.concatenate([pltpu.bitcast(X1B[j, pl.ds(w0, 128), :], jnp.bfloat16) for j in range(8)], axis=1)
            gbt = jnp.tile(MOD[...], (TM // 8, 1))
            out = (x1.astype(jnp.float32) + gbt * acc).astype(jnp.bfloat16)
            r0 = pl.multiple_of(r * TM, TM)
            OUTB[pl.ds(r0, TM), :] = out
            pltpu.make_async_copy(OUTB.at[pl.ds(r0, TM), :], out_hbm.at[0, pl.ds(r0, TM), :],
                                  sems.at[sem_i[0] + r]).start()
            return 0
        lax.fori_loop(0, S // TM, ffn_body, 0)
        for r in range(8):
            pltpu.make_async_copy(OUTB.at[pl.ds(TM * r, TM), :], out_hbm.at[0, pl.ds(TM * r, TM), :],
                                  sems.at[sem_i[0] + r]).wait()

    return kernel


def build(cfg=None):
    cfg = cfg or {}
    kernel = make_kernel(cfg)
    f32, bf16, u32 = jnp.float32, jnp.bfloat16, jnp.uint32
    V = pltpu.VMEM
    scratch = [
        V((8, SPAD, 128), bf16),
        V((NP, TM, D), bf16),
        V((D, 3 * D), bf16),
        V((16, 256, 128), f32), V((32, 256, 128), f32), V((32, 256, 128), f32),
        V((16, 256, 128), f32), V((32, 256, 128), f32), V((32, 256, 128), f32),
        V((NP, 264, 128), u32), V((NP, 264, 128), u32),
        V((D, D), bf16),
        V((NP, TM, D), f32),
        V((8, WPAD, 128), u32),
        V((8, WPAD, 128), u32),
        V((D, F), bf16), V((D, F), bf16), V((F, D), bf16),
        V((D, 6 * D), bf16),
        V((S, D), bf16),
        V((8, D), f32),
        pltpu.SemaphoreType.DMA((64,)),
    ]
    anyspec = pl.BlockSpec(memory_space=pl.ANY)
    return pl.pallas_call(
        kernel,
        out_shape=jax.ShapeDtypeStruct((1, S, D), bf16),
        in_specs=[anyspec] * 6 + [pl.BlockSpec(memory_space=pltpu.VMEM), anyspec],
        out_specs=anyspec,
        scratch_shapes=scratch,
        compiler_params=pltpu.CompilerParams(vmem_limit_bytes=cfg.get('vmem', 120 * 2 ** 20), flags=cfg.get('flags')),
    )


@jax.jit
def pallas_adaLN_cond__sliding_local_dilated__glu_gated_swiglu__prompt_kernel(
    A_x: jax.Array,
    A_wqkv: jax.Array,
    A_wo: jax.Array,
    B_x: jax.Array,
    B_w1: jax.Array,
    B_w3: jax.Array,
    B_w2: jax.Array,
    c: jax.Array,
    w_mod: jax.Array,
):
    del B_x
    return build({})(A_x, A_wqkv, A_wo, B_w1, B_w3, B_w2, c, w_mod)
```

```python
import functools
import jax
import jax.numpy as jnp
from jax import lax
from jax.experimental import pallas as pl
from jax.experimental.pallas import tpu as pltpu

S, D, F = 2048, 1024, 3584
NP = 8
NU = 4
TM = 256
LOG2E = 1.4426950408889634
QSCALE = (32 ** -0.5) * LOG2E
EPS = 1e-5
SPAD = 2064
WPAD = 1032


def zero_of(v):
    b = pltpu.bitcast(v, jnp.uint32)
    return (b >> 31) >> 1


def tie_lhs(h, ties):
    if not ties:
        return h
    K = h.shape[1]
    nk = K // 512 if K >= 512 else 1
    kw = 512 if K >= 512 else K
    rows = []
    for g in range(h.shape[0] // 16):
        blk = h[16 * g:16 * g + 16, :]
        if any((g, kh) in ties for kh in range(nk)):
            cols = []
            for kh in range(nk):
                a = blk[:, kh * kw:(kh + 1) * kw]
                if (g, kh) in ties:
                    a0 = pltpu.bitcast(pltpu.bitcast(a[:, :128], jnp.uint32) | ties[(g, kh)], jnp.bfloat16)
                    a = jnp.concatenate([a0, a[:, 128:]], axis=1)
                cols.append(a)
            blk = jnp.concatenate(cols, axis=1) if len(cols) > 1 else cols[0]
        rows.append(blk)
    return jnp.concatenate(rows, axis=0)


def layer_norm(x):
    mean = jnp.sum(x, axis=1, keepdims=True) * (1.0 / D)
    xc = x - mean
    var = jnp.sum(xc * xc, axis=1, keepdims=True) * (1.0 / D)
    return xc * lax.rsqrt(var + EPS)


def load_words_bf16(buf, p):
    parts = [pltpu.bitcast(buf.at[j].bitcast(jnp.uint32)[pl.ds(p, 128, stride=8), :], jnp.bfloat16)
             for j in range(8)]
    return jnp.concatenate(parts, axis=1)


def load_words(buf, p):
    return jnp.concatenate([buf.at[j].bitcast(jnp.uint32)[pl.ds(p, 128, stride=8), :] for j in range(8)], axis=1)


def unpack2(w):
    lo = pltpu.unpack_elementwise(w, index=0, packed_dtype=jnp.bfloat16, unpacked_dtype=jnp.float32)
    hi = pltpu.unpack_elementwise(w, index=1, packed_dtype=jnp.bfloat16, unpacked_dtype=jnp.float32)
    return lo, hi


def pack2(e, o):
    return pltpu.pack_elementwise([e, o], packed_dtype=jnp.bfloat16)


def tie_rhs(w, ties):
    if not ties:
        return w
    cols = []
    for j in range(w.shape[1] // 128):
        c = w[:, 128 * j:128 * (j + 1)]
        if any(k[1] == j for k in ties):
            rows = []
            for i in range(w.shape[0] // 16):
                b = c[16 * i:16 * i + 16]
                if (i, j) in ties:
                    b = pltpu.bitcast(pltpu.bitcast(b, jnp.uint32) | ties[(i, j)], jnp.bfloat16)
                rows.append(b)
            c = jnp.concatenate(rows, axis=0)
        cols.append(c)
    return jnp.concatenate(cols, axis=1)


def pin_words(w):
    acc = None
    for i in range(w.shape[0] // 8):
        for j in range(w.shape[1] // 128):
            b = w[8 * i:8 * i + 8, 128 * j:128 * (j + 1)]
            acc = b if acc is None else (acc | b)
    return (acc >> 31) >> 1


def store_words(buf_u32, p, val_bf16):
    wd = pltpu.bitcast(val_bf16, jnp.uint32)
    for j in range(8):
        buf_u32[j, pl.ds(p, 128, stride=8), :] = wd[:, 128 * j:128 * (j + 1)]
    return wd


def qdot(h, WQKV, R, p, t, u, ties, rties=None, split_pins=False):
    h = tie_lhs(h, ties)
    col = t * D + 256 * u
    r = jnp.dot(h, tie_rhs(WQKV[:, col:col + 256], rties), preferred_element_type=jnp.float32)
    pins = []
    marker = r[0:8, 0:128]
    if t == 0:
        r = r * QSCALE
    wd = pack2(r[0:128], r[128:256])
    off = 0 if t == 0 else 16
    for j in range(2):
        wt = wd[:, j * 128:(j + 1) * 128].T
        for hf in range(2):
            rho = 2 * p + hf
            val = pltpu.unpack_elementwise(wt, index=hf, packed_dtype=jnp.bfloat16, unpacked_dtype=jnp.float32)
            for hh in range(4):
                R[off + rho, pl.ds(4 * j + hh, 32, stride=8), :] = val[32 * hh:32 * hh + 32]
            if t > 0 and not (isinstance(p, int) and p == 0):
                sv = pltpu.roll(val, 1, 1)
                for hh in range(4):
                    R[rho, pl.ds(4 * j + hh, 32, stride=8), :] = sv[32 * hh:32 * hh + 32]
                val = sv
            pins.append(pltpu.bitcast(val[120:128], jnp.uint32))
    if split_pins:
        return marker, [(x >> 31) >> 1 for x in pins]
    pin = functools.reduce(lambda a, b: a | b, pins)
    return marker, (pin >> 31) >> 1


def attend_steps(RQ, RK, RV, p):
    lane = lax.broadcasted_iota(jnp.int32, (8, 128), 1)
    markers = []
    Ps = []
    for hf in range(2):
        rho = 2 * p + hf
        q = RQ[rho].reshape(32, 8, 128)
        Ls = []
        for w in range(8):
            kap = rho - 2 * w
            kk = RK[16 + kap].reshape(32, 8, 128)
            L = jnp.sum(q * kk, axis=0)
            if isinstance(kap, int):
                if kap < 0:
                    L = jnp.where(lane <= 0, -1e9, L)
            elif w > 0:
                thr = jnp.where(kap < 0, 0, -1)
                L = jnp.where(lane <= thr, -1e9, L)
            Ls.append(L)
            markers.append(zero_of(L))
        m = functools.reduce(jnp.maximum, Ls)
        es = [jnp.exp2(L - m) for L in Ls]
        ssum = functools.reduce(jnp.add, es)
        inv = 1.0 / ssum
        Ps.append([e * inv for e in es])
        markers.append(zero_of(inv))
    words = []
    for dg in range(16):
        ws = []
        for d in range(2 * dg, 2 * dg + 2):
            os_ = []
            for hf in range(2):
                rho = 2 * p + hf
                o = None
                for w in range(8):
                    kap = rho - 2 * w
                    vv = RV[16 + kap, 8 * d:8 * d + 8, :]
                    tt = Ps[hf][w] * vv
                    o = tt if o is None else o + tt
                os_.append(o)
            ws.append(pltpu.pack_elementwise(os_, packed_dtype=jnp.bfloat16))
        words += ws
        markers.append(zero_of(ws[0] | ws[1]))
    return markers, words


def store_o(OS, p, words, throttle):
    if throttle is not None:
        words = [w | throttle for w in words]
    OS[p, 0:256, :] = jnp.concatenate(words, axis=0)


def out_dot(OS, p, WO, u, rties=None):
    parts = []
    for jj in range(2):
        rows = [OS[p, pl.ds(4 * jj + hh, 32, stride=8), :] for hh in range(4)]
        nat = jnp.concatenate(rows, axis=0)
        parts.append(nat.T)
    lo, hi = unpack2(jnp.concatenate(parts, axis=1))
    lhs = jnp.concatenate([lo, hi], axis=0).astype(jnp.bfloat16)
    rhs = tie_rhs(WO[256 * u:256 * u + 256, :], rties)
    return jnp.dot(lhs, rhs, preferred_element_type=jnp.float32)


def spread(markers, slots, lo, hi):
    ties = {}
    n = len(markers)
    for i, mk in enumerate(markers):
        t, kh, g = slots[lo + (i * (hi - lo)) // n]
        ties.setdefault(t, {})
        key = (g, kh)
        ties[t][key] = mk if key not in ties[t] else (ties[t][key] | mk)
    return ties


def spread_rhs_out(markers, t_lo, t_hi):
    ties = {}
    n = len(markers)
    used = {}
    for m, mk in enumerate(markers):
        ts = t_lo + (m * (t_hi - t_lo)) // n
        ps, ii = ts // 8, 7 - (ts % 8)
        k = used.get(ts, 0)
        used[ts] = k + 1
        k = k % 4
        key = (ii + 8 * (k // 2), 2 * ps + (k % 2))
        ties[key] = mk if key not in ties else (ties[key] | mk)
    return ties


def rhs_key(kind, ts, k):
    ps, ii = ts // 8, 7 - (ts % 8)
    if kind == 'qkv':
        return (32 * (ps % 2) + 8 * k + ii, ps // 2)
    return (ii + 8 * (k // 2), 2 * ps + (k % 2))


class Ties:
    def __init__(self, kinds):
        self.kinds = kinds
        self.t = [dict() for _ in kinds]
        self.used = {}

    def add(self, gslot, z):
        d, ts = gslot // 32, gslot % 32
        d = min(d, len(self.kinds) - 1)
        k = self.used.get((d, ts), 0)
        self.used[(d, ts)] = k + 1
        key = rhs_key(self.kinds[d], ts, k % 4)
        cur = self.t[d].get(key)
        self.t[d][key] = z if cur is None else (cur | z)

    def spread(self, markers, lo, hi):
        n = len(markers)
        for m, mk in enumerate(markers):
            self.add(lo + (m * (hi - lo)) // n, mk)

    def get(self, d):
        return self.t[d]


SLOTS_QKV = [(t, kh, g) for t in range(3) for kh in range(2) for g in range(16)]


def make_kernel(cfg):
    unroll_u = cfg.get('unroll_u', 1)
    gemv_u = cfg.get('gemv_u', 2)
    static_u = cfg.get('static_u', False)
    t1_row, t1_col = cfg.get('t1_thr', (0, 768))
    at_lo, at_hi, at3_hi = cfg.get('at_lo', 2), cfg.get('at_hi', 82), cfg.get('at3_hi', 90)
    pin_q, pin_k, pin_v, pin_v_same = cfg.get('pin_q', 20), cfg.get('pin_k', 28), cfg.get('pin_v', 12), cfg.get('pin_v_same', 0)
    g_per = cfg.get('g_per', 3)
    ffn_tm = cfg.get('ffn_tm', 256)
    ffn_mode = cfg.get('ffn_mode', 'flat')
    order3 = cfg.get('order3', (2, 1, 0))
    pin_sl = cfg.get('pin_sl', (8, 16, 24, 31))
    pin_sl3 = cfg.get('pin_sl3', (8, 16, 24, 31))
    t_w, t_lo, t_len, t_thr = cfg.get('t_w', 48), cfg.get('t_lo', 4), cfg.get('t_len', 44), cfg.get('t_thr', 24)

    import contextlib
    def scope(name):
        return jax.named_scope(name) if cfg.get('scopes') else contextlib.nullcontext()

    def kernel(x_hbm, wqkv_hbm, wo_hbm, w1_hbm, w3_hbm, w2_hbm, c_hbm, wmod_hbm, out_hbm,
               CV, XB, HP, WQKV, RQ0, RK0, RV0, RQ1, RK1, RV1, OS0, OS1, WO, ACC, H2T, X1B,
               W1, W3, W2, WMOD, OUTB, MOD2, sems):
        Rset = [(RQ0, RK0, RV0), (RQ1, RK1, RV1)]
        OSs = [OS0, OS1]
        sem_i = [0]

        def new_copy(src, dst):
            i = sem_i[0]
            sem_i[0] += 1
            return pltpu.make_async_copy(src, dst, sems.at[i])

        cp_c = new_copy(c_hbm, CV)
        cp_x = [new_copy(x_hbm.at[0, :, pl.ds(128 * j, 128)], XB.at[j, pl.ds(0, S), :]) for j in range(8)]
        cp_mod01 = [new_copy(wmod_hbm.at[:, pl.ds(512 * i, 512)], WMOD.at[:, pl.ds(512 * i, 512)]) for i in range(4)]
        cp_mod = [None, None] + [new_copy(wmod_hbm.at[:, pl.ds(1024 * i, 1024)], WMOD.at[:, pl.ds(1024 * i, 1024)]) for i in range(2, 6)]
        cp_qkv = [[new_copy(wqkv_hbm.at[:, pl.ds(t * D + 256 * u, 256)], WQKV.at[:, pl.ds(t * D + 256 * u, 256)])
                   for t in range(3)] for u in range(NU)]
        cp_wo = new_copy(wo_hbm, WO)
        cp_w1 = new_copy(w1_hbm, W1)
        cp_w3 = new_copy(w3_hbm, W3)
        cp_w2 = new_copy(w2_hbm, W2)


        cp_c.start()
        for c_ in cp_x:
            c_.start()
        for c_ in cp_mod01:
            c_.start()
        for u in range(NU):
            for c_ in cp_qkv[u]:
                c_.start()
            if u == 1:
                cp_wo.start()
        for i in range(2, 6):
            cp_mod[i].start()
        cp_w1.start()
        cp_w3.start()
        cp_w2.start()
        with scope('wait_x'):
            cp_c.wait()
            for c_ in cp_x:
                c_.wait()
        cv = CV[...].astype(jnp.float32)
        sc = (cv * jax.nn.sigmoid(cv)).astype(jnp.bfloat16)
        sc16 = jnp.broadcast_to(sc, (16, D))
        with scope('ln1'):
            for p in range(NP):
                lo, hi = unpack2(load_words(XB, p))
                ACC[p] = layer_norm(jnp.concatenate([lo, hi], axis=0))
        m01 = []
        with scope('mod'):
            for i in range(4):
                cp_mod01[i].wait()
                m01.append(jnp.dot(sc16, WMOD[:, 512 * i:512 * (i + 1)], preferred_element_type=jnp.float32)[0:8])
        sa = jnp.concatenate(m01[0:2], axis=1)
        a1 = 1.0 + jnp.concatenate(m01[2:4], axis=1)
        with scope('wait_qkv0'):
            for c_ in cp_qkv[0]:
                c_.wait()

        sa_t = jnp.tile(sa, (TM // 8, 1))
        a1_t = jnp.tile(a1, (TM // 8, 1))
        with scope('unit0'):
            for p in range(NP):
                h = (ACC[p] * a1_t + sa_t).astype(jnp.bfloat16)
                HP[p] = h
                for t in range(3):
                    qdot(h, WQKV, Rset[0][t], p, t, 0, None)

        with scope('wait_u'):
            for u in range(1, NU):
                for c_ in cp_qkv[u]:
                    c_.wait()
            cp_wo.wait()
        carry = []

        def gemv_piece(i):
            c0 = 128 * i
            g2 = jnp.dot(sc16, WMOD[:, pl.ds(2048 + c0, 128)], preferred_element_type=jnp.float32)
            MOD2[:, pl.ds(c0, 128)] = g2[0:8, :]

        with scope('units'):
          for u in range(1, NU):
            Rw = Rset[u % 2]
            Rr = Rset[(u - 1) % 2]
            OS = OSs[(u - 1) % 2]
            with_out = u <= 2
            if u == gemv_u:
                for i in range(2, 6):
                    cp_mod[i].wait()
                carry = []
            for p in range(NP):
                markers, words = attend_steps(Rr[0], Rr[1], Rr[2], p)
                h = HP[p]
                kinds = ['qkv'] * 3 + (['out'] if with_out else [])
                T = Ties(kinds)
                lt = spread(markers, SLOTS_QKV, at_lo, at_hi if with_out else at3_hi)
                for slot, z in carry:
                    T.add(slot, z)
                carry = []
                order = (0, 1, 2) if with_out else order3
                ms = []
                for i, t in enumerate(order):
                    m, pns = qdot(h, WQKV, Rw[t], p, t, u, lt.get(i), T.get(i), True)
                    ms.append(m)
                    if u == gemv_u:
                        gemv_piece(4 * p + i)
                    for pn, sl in zip(pns, pin_sl if with_out else pin_sl3):
                        tgt = 32 * (i + 1) + sl
                        if tgt < 32 * len(kinds):
                            T.add(tgt, pn)
                        else:
                            carry.append((tgt - 32 * len(kinds), pn))
                store_o(OS, p, words, zero_of(ms[2]) if with_out else None)
                if with_out:
                    res = out_dot(OS, p, WO, u - 1, T.get(3))
                    if u == 1:
                        ACC[p] = res
                    else:
                        ACC[p] += res
                    if u == gemv_u:
                        gemv_piece(4 * p + 3)

        with scope('wait_t'):
            cp_w1.wait()
            cp_w3.wait()
            cp_w2.wait()

        ga_t = jnp.tile(MOD2[:, 0:1024], (128 // 8, 1))
        T = Ties(['out'] * 16)
        at_done = {}
        with scope('t'):
            for d in range(16):
                for p in range(NP):
                    if p not in at_done and (p * t_w) // 32 <= d:
                        markers, words = attend_steps(RQ1, RK1, RV1, p)
                        T.spread(markers, p * t_w + t_lo, p * t_w + t_lo + t_len)
                        at_done[p] = words
                res = out_dot(OS0 if d < 8 else OS1, d % 8, WO, 2 if d < 8 else 3, T.get(d))
                for p in range(NP):
                    endslot = p * t_w + t_lo + t_len
                    if at_done.get(p) is not None and p in at_done and (endslot + t_thr) // 32 <= d:
                        store_o(OS1, p, at_done[p], zero_of(res[0:8, 0:128]))
                        at_done[p] = None
                if d < 8:
                    ACC[d] += res
                else:
                    p = d - 8
                    a = ACC[p] + res
                    lo, hi = unpack2(load_words(XB, p))
                    x1w = pack2(lo + ga_t * a[0:128], hi + ga_t * a[128:256])
                    for j in range(8):
                        X1B[j, pl.ds(p, 128, stride=8), :] = x1w[:, 128 * j:128 * (j + 1)]

        TMF = ffn_tm
        NT = S // TMF
        WR = TMF // 2

        def ln2_tile(r0w, nw):
            x1 = jnp.concatenate([pltpu.bitcast(X1B[j, pl.ds(r0w, nw), :], jnp.bfloat16) for j in range(8)], axis=1)
            b1 = jnp.tile(1.0 + MOD2[:, 2048:3072], (2 * nw // 8, 1))
            sb = jnp.tile(MOD2[:, 1024:2048], (2 * nw // 8, 1))
            return layer_norm(x1.astype(jnp.float32)) * b1 + sb

        with scope('ln2_0'):
            H2T[0] = ln2_tile(0, WR).astype(jnp.bfloat16)

        TN = 512
        if ffn_mode == 'flat':
            def ffn_body(r, _):
                w0 = pl.multiple_of(r * WR, WR)
                h = H2T[r % 2]
                wn = pl.multiple_of(jnp.minimum(r + 1, NT - 1) * WR, WR)
                hn = ln2_tile(wn, WR)
                H2T[(r + 1) % 2] = hn.astype(jnp.bfloat16)
                hb = pltpu.bitcast(hn, jnp.uint32)
                ng = TMF // 16
                pins = [pin_words(hb[16 * g:16 * g + 16]) for g in range(ng)]
                acc = None
                for j in range(F // TN):
                    hj = h
                    if j == 2:
                        hj = tie_lhs(h, {(g, 0): pins[g] for g in range(ng)})
                    g = jnp.dot(hj, W1[:, j * TN:(j + 1) * TN], preferred_element_type=jnp.float32)
                    up = jnp.dot(h, W3[:, j * TN:(j + 1) * TN], preferred_element_type=jnp.float32)
                    a = (g * jax.nn.sigmoid(g) * up).astype(jnp.bfloat16)
                    o = jnp.dot(a, W2[j * TN:(j + 1) * TN, :], preferred_element_type=jnp.float32)
                    acc = o if acc is None else acc + o
                x1 = jnp.concatenate([pltpu.bitcast(X1B[j, pl.ds(w0, WR), :], jnp.bfloat16) for j in range(8)], axis=1)
                gbt = jnp.tile(MOD2[:, 3072:4096], (TMF // 8, 1))
                out = (x1.astype(jnp.float32) + gbt * acc).astype(jnp.bfloat16)
                r0 = pl.multiple_of(r * TMF, TMF)
                OUTB[pl.ds(r0, TMF), :] = out
                pltpu.make_async_copy(OUTB.at[pl.ds(r0, TMF), :], out_hbm.at[0, pl.ds(r0, TMF), :],
                                      sems.at[sem_i[0] + r]).start()
                return 0
            with scope('ffn'):
                lax.fori_loop(0, NT, ffn_body, 0)
        else:
            TH = F // 2
            TC = 256

            def epilogue(rp, k):
                w0 = pl.multiple_of(rp * 128 + k * 64, 64)
                x1 = jnp.concatenate([pltpu.bitcast(X1B[j, pl.ds(w0, 64), :], jnp.bfloat16) for j in range(8)], axis=1)
                gbt = jnp.tile(MOD2[:, 3072:4096], (128 // 8, 1))
                a0 = pl.multiple_of(k * 128, 128)
                out = (x1.astype(jnp.float32) + gbt * ACC[rp % 2, pl.ds(a0, 128), :]).astype(jnp.bfloat16)
                r0 = pl.multiple_of(rp * 256 + k * 128, 128)
                OUTB[pl.ds(r0, 128), :] = out
                return out

            def ffn_body(i, _):
                r = i // 2
                k = i % 2
                h = H2T[r % 2]
                wn = pl.multiple_of(jnp.minimum(r + 1, 7) * 128 + k * 64, 64)
                hn = ln2_tile(wn, 64)
                H2T[(r + 1) % 2, pl.ds(pl.multiple_of(k * 128, 128), 128), :] = hn.astype(jnp.bfloat16)
                hb = pltpu.bitcast(hn, jnp.uint32)
                pins = [pin_words(hb[16 * g:16 * g + 16]) for g in range(8)]
                rp = jnp.maximum(r - 1, 0)
                eo = epilogue(rp, k)
                eb = pltpu.bitcast(eo, jnp.uint32)
                pins2 = [pin_words(eb[8 * g:8 * g + 8]) for g in range(8)]
                c0 = pl.multiple_of(k * TH, 128)
                acc = None
                for j in range(TH // TC):
                    hj = h
                    if j == 1:
                        hj = tie_lhs(h, {(2 * g, 0): pins[g] for g in range(8)})
                    if j == 3:
                        hj = tie_lhs(h, {(2 * g, 0): pins2[g] for g in range(8)})
                    cj = pl.ds(c0 + j * TC, TC)
                    g = jnp.dot(hj, W1[:, cj], preferred_element_type=jnp.float32)
                    up = jnp.dot(h, W3[:, cj], preferred_element_type=jnp.float32)
                    a = (g * jax.nn.sigmoid(g) * up).astype(jnp.bfloat16)
                    o = jnp.dot(a, W2[cj, :], preferred_element_type=jnp.float32)
                    acc = o if acc is None else acc + o
                prev = ACC[r % 2]
                ACC[r % 2] = acc + jnp.where(k == 0, 0.0, prev)

                @pl.when((k == 1) & (r >= 1))
                def _():
                    r0 = pl.multiple_of(rp * 256, 256)
                    pltpu.make_async_copy(OUTB.at[pl.ds(r0, 256), :], out_hbm.at[0, pl.ds(r0, 256), :],
                                          sems.at[sem_i[0] + rp]).start()
                return 0
            with scope('ffn'):
                lax.fori_loop(0, 16, ffn_body, 0)
            with scope('ffn_last'):
                epilogue(7, 0)
                epilogue(7, 1)
                pltpu.make_async_copy(OUTB.at[pl.ds(7 * 256, 256), :], out_hbm.at[0, pl.ds(7 * 256, 256), :],
                                      sems.at[sem_i[0] + 7]).start()
            NT, TMF = 8, 256
        with scope('tail'):
          for r in range(NT):
            pltpu.make_async_copy(OUTB.at[pl.ds(TMF * r, TMF), :], out_hbm.at[0, pl.ds(TMF * r, TMF), :],
                                  sems.at[sem_i[0] + r]).wait()

    return kernel


def build(cfg=None):
    cfg = cfg or {}
    kernel = make_kernel(cfg)
    f32, bf16, u32 = jnp.float32, jnp.bfloat16, jnp.uint32
    V = pltpu.VMEM
    scratch = [
        V((1, D), bf16),
        V((8, SPAD, 128), bf16),
        V((NP, TM, D), bf16),
        V((D, 3 * D), bf16),
        V((16, 256, 128), f32), V((32, 256, 128), f32), V((32, 256, 128), f32),
        V((16, 256, 128), f32), V((32, 256, 128), f32), V((32, 256, 128), f32),
        V((NP, 264, 128), u32), V((NP, 264, 128), u32),
        V((D, D), bf16),
        V((NP, TM, D), f32),
        V((2, cfg.get('ffn_tm', 256), D), bf16),
        V((8, WPAD, 128), u32),
        V((D, F), bf16), V((D, F), bf16), V((F, D), bf16),
        V((D, 6 * D), bf16),
        V((S, D), bf16),
        V((8, 4 * D), f32),
        pltpu.SemaphoreType.DMA((64,)),
    ]
    anyspec = pl.BlockSpec(memory_space=pl.ANY)
    return pl.pallas_call(
        kernel,
        out_shape=jax.ShapeDtypeStruct((1, S, D), bf16),
        in_specs=[anyspec] * 6 + [anyspec, anyspec],
        out_specs=anyspec,
        scratch_shapes=scratch,
        compiler_params=pltpu.CompilerParams(vmem_limit_bytes=cfg.get('vmem', 120 * 2 ** 20), flags=cfg.get('flags')),
    )


@jax.jit
def pallas_adaLN_cond__sliding_local_dilated__glu_gated_swiglu__prompt_kernel(
    A_x: jax.Array,
    A_wqkv: jax.Array,
    A_wo: jax.Array,
    B_x: jax.Array,
    B_w1: jax.Array,
    B_w3: jax.Array,
    B_w2: jax.Array,
    c: jax.Array,
    w_mod: jax.Array,
):
    del B_x
    return build({'ffn_tm': 128})(A_x, A_wqkv, A_wo, B_w1, B_w3, B_w2, c, w_mod)
```

```python
import contextlib
import functools
import jax
import jax.numpy as jnp
from jax import lax
from jax.experimental import pallas as pl
from jax.experimental.pallas import tpu as pltpu

S, D, F = 2048, 1024, 3584
NP = 8
NU = 4
TM = 256
LOG2E = 1.4426950408889634
QSCALE = (32 ** -0.5) * LOG2E
EPS = 1e-5
SPAD = 2064
WPAD = 1032
f32, bf16, u32 = jnp.float32, jnp.bfloat16, jnp.uint32


def zero_of(v):
    b = pltpu.bitcast(v, u32)
    return (b >> 31) >> 1


def unpack2(w):
    lo = pltpu.unpack_elementwise(w, index=0, packed_dtype=bf16, unpacked_dtype=f32)
    hi = pltpu.unpack_elementwise(w, index=1, packed_dtype=bf16, unpacked_dtype=f32)
    return lo, hi


def pack2(e, o):
    return pltpu.pack_elementwise([e, o], packed_dtype=bf16)


def or_all(vals):
    return functools.reduce(lambda a, b: a | b, vals)


def tie_lhs(h, ties):
    if not ties:
        return h
    K = h.shape[1]
    nk = K // 512 if K >= 512 else 1
    kw = 512 if K >= 512 else K
    rows = []
    for g in range(h.shape[0] // 16):
        blk = h[16 * g:16 * g + 16, :]
        if any((g, kh) in ties for kh in range(nk)):
            cols = []
            for kh in range(nk):
                a = blk[:, kh * kw:(kh + 1) * kw]
                if (g, kh) in ties:
                    a0 = pltpu.bitcast(pltpu.bitcast(a[:, :128], u32) | ties[(g, kh)], bf16)
                    a = jnp.concatenate([a0, a[:, 128:]], axis=1)
                cols.append(a)
            blk = jnp.concatenate(cols, axis=1) if len(cols) > 1 else cols[0]
        rows.append(blk)
    return jnp.concatenate(rows, axis=0)


def tie_rhs(w, ties):
    if not ties:
        return w
    cols = []
    for j in range(w.shape[1] // 128):
        c = w[:, 128 * j:128 * (j + 1)]
        if any(k[1] == j for k in ties):
            rows = []
            for i in range(w.shape[0] // 16):
                b = c[16 * i:16 * i + 16]
                if (i, j) in ties:
                    b = pltpu.bitcast(pltpu.bitcast(b, u32) | ties[(i, j)], bf16)
                rows.append(b)
            c = jnp.concatenate(rows, axis=0)
        cols.append(c)
    return jnp.concatenate(cols, axis=1)


def rhs_key(kind, ts, k):
    ps, ii = ts // 8, 7 - (ts % 8)
    if kind == 'qkv':
        return (32 * (ps % 2) + 8 * k + ii, ps // 2)
    return (ii + 8 * (k // 2), 2 * ps + (k % 2))


class Ties:
    def __init__(self, kinds):
        self.kinds = kinds
        self.t = [dict() for _ in kinds]
        self.used = {}

    def add(self, gslot, z):
        gslot = max(gslot, 0)
        d, ts = gslot // 32, gslot % 32
        if d >= len(self.kinds):
            return False
        k = self.used.get((d, ts), 0)
        self.used[(d, ts)] = k + 1
        key = rhs_key(self.kinds[d], ts, k % 4)
        cur = self.t[d].get(key)
        self.t[d][key] = z if cur is None else (cur | z)
        return True

    def spread(self, markers, lo, hi):
        n = len(markers)
        for m, mk in enumerate(markers):
            self.add(lo + (m * (hi - lo)) // n, mk)

    def get(self, d):
        return self.t[d]


def spread_lhs(markers, ndots, lo, hi):
    slots = [(t, kh, g) for t in range(ndots) for kh in range(2) for g in range(16)]
    ties = {}
    n = len(markers)
    for i, mk in enumerate(markers):
        t, kh, g = slots[lo + (i * (hi - lo)) // n]
        ties.setdefault(t, {})
        key = (g, kh)
        ties[t][key] = mk if key not in ties[t] else (ties[t][key] | mk)
    return ties


def ln_stats(x):
    mean = jnp.sum(x, axis=1, keepdims=True) * (1.0 / D)
    xc = x - mean
    var = jnp.sum(xc * xc, axis=1, keepdims=True) * (1.0 / D)
    return xc, lax.rsqrt(var + EPS)


def layer_norm(x):
    xc, r = ln_stats(x)
    return xc * r


def load_words(buf, p):
    return jnp.concatenate([buf.at[j].bitcast(u32)[pl.ds(p, 128, stride=8), :] for j in range(8)], axis=1)


def store_heads(R, idx, j, val):
    for hh in range(4):
        R[idx, pl.ds(4 * j + hh, 32, stride=8), :] = val[32 * hh:32 * hh + 32]


def qdot(h, WQKV, R, p, t, u, ties, rties):
    h = tie_lhs(h, ties)
    col = t * D + 256 * u
    r = jnp.dot(h, tie_rhs(WQKV[:, col:col + 256], rties), preferred_element_type=f32)
    marker = r[0:8, 0:128]
    if t == 0:
        r = r * QSCALE
    wd = pack2(r[0:128], r[128:256])
    off = 0 if t == 0 else 16
    pins = []
    for j in range(2):
        wt = wd[:, j * 128:(j + 1) * 128].T
        for hf, val in enumerate(unpack2(wt)):
            rho = 2 * p + hf
            store_heads(R, off + rho, j, val)
            if t > 0 and p > 0:
                val = pltpu.roll(val, 1, 1)
                store_heads(R, rho, j, val)
            pins.append((pltpu.bitcast(val[120:128], u32) >> 31) >> 1)
    return marker, pins


def attend_steps(RQ, RK, RV, p):
    lane = lax.broadcasted_iota(jnp.int32, (8, 128), 1)
    markers = []
    Ps = []
    for hf in range(2):
        rho = 2 * p + hf
        q = RQ[rho].reshape(32, 8, 128)
        Ls = []
        for w in range(8):
            kap = rho - 2 * w
            kk = RK[16 + kap].reshape(32, 8, 128)
            L = jnp.sum(q * kk, axis=0)
            if kap < 0:
                L = jnp.where(lane <= 0, -1e9, L)
            Ls.append(L)
            markers.append(zero_of(L))
        m = functools.reduce(jnp.maximum, Ls)
        es = [jnp.exp2(L - m) for L in Ls]
        ssum = functools.reduce(jnp.add, es)
        inv = 1.0 / ssum
        Ps.append([e * inv for e in es])
        markers.append(zero_of(inv))
    words = []
    for dg in range(16):
        ws = []
        for d in range(2 * dg, 2 * dg + 2):
            os_ = []
            for hf in range(2):
                rho = 2 * p + hf
                o = None
                for w in range(8):
                    kap = rho - 2 * w
                    tt = Ps[hf][w] * RV[16 + kap, 8 * d:8 * d + 8, :]
                    o = tt if o is None else o + tt
                os_.append(o)
            ws.append(pack2(os_[0], os_[1]))
        words += ws
        markers.append(zero_of(ws[0] | ws[1]))
    return markers, words


def store_o(OS, p, words, throttle):
    if throttle is not None:
        words = [w | throttle for w in words]
    OS[p, 0:256, :] = jnp.concatenate(words, axis=0)


def out_dot(OS, p, WO, u, rties):
    parts = []
    for jj in range(2):
        rows = [OS[p, pl.ds(4 * jj + hh, 32, stride=8), :] for hh in range(4)]
        parts.append(jnp.concatenate(rows, axis=0).T)
    lo, hi = unpack2(jnp.concatenate(parts, axis=1))
    lhs = jnp.concatenate([lo, hi], axis=0).astype(bf16)
    rhs = tie_rhs(WO[256 * u:256 * u + 256, :], rties)
    return jnp.dot(lhs, rhs, preferred_element_type=f32)


def make_kernel(cfg):
    at_lo, at_hi, at3_hi = cfg.get('at_lo', 2), cfg.get('at_hi', 82), cfg.get('at3_hi', 90)
    pin_sl = cfg.get('pin_sl', (8, 16, 24, 31))
    t_w, t_lo, t_len, t_thr = cfg.get('t_w', 48), cfg.get('t_lo', 4), cfg.get('t_len', 44), cfg.get('t_thr', 24)
    u1_back, u1_len = cfg.get('u1_back', 36), cfg.get('u1_len', 80)
    ffn_tm = cfg.get('ffn_tm', 128)
    ln_pins = cfg.get('ln_pins', 16)
    nat_lo, nat_hi = cfg.get('nat_lo', 10), cfg.get('nat_hi', 50)

    def scope(name):
        return jax.named_scope(name) if cfg.get('scopes') else contextlib.nullcontext()

    def kernel(x_hbm, wqkv_hbm, wo_hbm, w1_hbm, w3_hbm, w2_hbm, c_hbm, wmod_hbm, out_hbm,
               CV, XB, HB, QN, BQ, HP, WQKV, RQ0, RK0, RV0, RQ1, RK1, RV1, OS0, OS1, WO, ACC, H2T, X1B,
               W1, W3, W2, WMOD, OUTB, MOD1, MOD2, sems):
        Rset = [(RQ0, RK0, RV0), (RQ1, RK1, RV1)]
        OSs = [OS0, OS1]
        XN = OUTB
        sem_i = [0]

        def new_copy(src, dst):
            i = sem_i[0]
            sem_i[0] += 1
            return pltpu.make_async_copy(src, dst, sems.at[i])

        def colcopy(src, dst, c0, n):
            return new_copy(src.at[:, pl.ds(c0, n)], dst.at[:, pl.ds(c0, n)])

        cp_c = new_copy(c_hbm, CV)
        cp_ca = [colcopy(wmod_hbm, WMOD, 1024 + 512 * i, 512) for i in range(2)]
        cp_sa = colcopy(wmod_hbm, WMOD, 0, 1024)
        cp_xn = [new_copy(x_hbm.at[0, pl.ds(TM * r, TM), :], XN.at[pl.ds(TM * r, TM), :]) for r in range(8)]
        cp_w = {(t, u): colcopy(wqkv_hbm, WQKV, t * D + 256 * u, 256) for t in range(3) for u in range(NU)}
        cp_wo = new_copy(wo_hbm, WO)
        cp_xb = [new_copy(x_hbm.at[0, :, pl.ds(128 * j, 128)], XB.at[j, pl.ds(0, S), :]) for j in range(8)]
        cp_mod2 = colcopy(wmod_hbm, WMOD, 2048, 4096)
        cp_ffn = [new_copy(w1_hbm, W1), new_copy(w3_hbm, W3), new_copy(w2_hbm, W2)]

        for c_ in ([cp_c] + cp_ca + [cp_xn[0], cp_xn[1], cp_w[0, 0], cp_w[0, 1]] + cp_xn[2:] + [cp_sa]
                   + [cp_w[1, 0], cp_w[2, 0], cp_w[1, 1], cp_w[2, 1], cp_wo]
                   + [cp_w[t, u] for u in (2, 3) for t in range(3)] + cp_xb + [cp_mod2] + cp_ffn):
            c_.start()

        with scope('mod_ca'):
            cp_c.wait()
            cv = CV[...].astype(f32)
            sc = (cv * jax.nn.sigmoid(cv)).astype(bf16)
            sc16 = jnp.broadcast_to(sc, (16, D))
            for i in range(2):
                cp_ca[i].wait()
                m = jnp.dot(sc16, WMOD[:, 1024 + 512 * i:1024 + 512 * (i + 1)], preferred_element_type=f32)
                MOD1[:, 1024 + 512 * i:1024 + 512 * (i + 1)] = 1.0 + m[0:8]

        def ln_nat(r):
            xc, rs = ln_stats(XN[pl.ds(TM * r, TM), :].astype(f32))
            hm = (xc * rs) * jnp.tile(MOD1[:, 1024:2048], (TM // 8, 1))
            h16 = hm.astype(bf16)
            for j in range(8):
                HB[j, pl.ds(TM * r, TM), :] = h16[:, 128 * j:128 * (j + 1)]
            hb = pltpu.bitcast(hm[:, 896:1024], u32)
            rows = TM // ln_pins
            return [(or_all([hb[rows * g + 8 * i:rows * g + 8 * i + 8] for i in range(rows // 8)]) >> 31) >> 1
                    for g in range(ln_pins)]

        def qnat(r, u, rties):
            hn = jnp.concatenate([HB[j, pl.ds(TM * r, TM), :] for j in range(8)], axis=1)
            res = jnp.dot(hn, tie_rhs(WQKV[:, 256 * u:256 * u + 256], rties), preferred_element_type=f32)
            res = (res * QSCALE).astype(bf16)
            for j in range(2):
                QN[2 * u + j, pl.ds(TM * r, TM), :] = res[:, 128 * j:128 * (j + 1)]

        def sa_piece(i):
            m = jnp.dot(sc16, WMOD[:, 128 * i:128 * (i + 1)], preferred_element_type=f32)
            MOD1[:, 128 * i:128 * (i + 1)] = m[0:8]

        with scope('nat0'):
            cp_xn[0].wait()
            ln_nat(0)
            cp_xn[1].wait()
            ln_nat(1)
            cp_w[0, 0].wait()
            qnat(0, 0, None)
            qnat(1, 0, None)

        def nat_region(waits, seq, extra=None):
            for c_ in waits:
                c_.wait()
            T = Ties(['qkv'] * (2 * len(seq)))
            for i, (r, ln_r) in enumerate(seq):
                if ln_r is not None:
                    T.spread(ln_nat(ln_r), 64 * i + nat_lo, 64 * i + nat_hi)
                for k, (rr, u) in enumerate(r):
                    qnat(rr, u, T.get(2 * i + k))
                    if extra:
                        extra(2 * i + k)

        with scope('nat1'):
            nat_region([cp_w[0, 1], cp_xn[2]], [([(0, 1), (1, 1)], 2)])
        with scope('nat2'):
            nat_region([cp_xn[3], cp_xn[4]], [([(2, 0), (2, 1)], 3), ([(3, 0), (3, 1)], 4)])
        with scope('nat3'):
            nat_region(cp_xn[5:], [([(4, 0), (4, 1)], 5), ([(5, 0), (5, 1)], 6)])
        with scope('nat4'):
            def sa_extra(d):
                for i in range(2 * d, 2 * d + 2):
                    sa_piece(i)
            nat_region([cp_sa], [([(6, 0), (6, 1)], 7), ([(7, 0), (7, 1)], None)], sa_extra)

        for c_ in [cp_w[1, 0], cp_w[2, 0]]:
            c_.wait()
        sa_t = jnp.tile(MOD1[:, 0:1024], (128 // 8, 1))

        def make_hp(p):
            lo, hi = unpack2(load_words(HB, p))
            h = jnp.concatenate([lo + sa_t, hi + sa_t], axis=0).astype(bf16)
            HP[p] = h
            return h

        def bias_piece(i):
            sa16 = jnp.tile(MOD1[:, 0:1024], (2, 1)).astype(bf16)
            b = jnp.dot(sa16, WQKV[:, 128 * i:128 * (i + 1)], preferred_element_type=f32)[0:8] * QSCALE
            BQ[i] = jnp.tile(b, (16, 1)).T

        def rl_piece(u, j, p):
            w = QN.at[2 * u + j].bitcast(u32)[pl.ds(p, 128, stride=8), :]
            wt = w.T
            last = None
            for hf, val in enumerate(unpack2(wt)):
                val = val + BQ[2 * u + j]
                store_heads(Rset[u][0], 2 * p + hf, j, val)
                last = val
            return (pltpu.bitcast(last[120:128], u32) >> 31) >> 1

        with scope('kv0'):
            T = Ties(['qkv'] * 16)
            pieces = [(u, j, p) for u in range(2) for p in range(NP) for j in range(2)]
            for p in range(NP):
                if p == 1:
                    T.spread([rl_piece(*pc) for pc in pieces], 96, 500)
                h = make_hp(p)
                for i, t in enumerate((1, 2)):
                    m, pns = qdot(h, WQKV, Rset[0][t], p, t, 0, None, T.get(2 * p + i))
                    if p == 0:
                        bias_piece(2 * i)
                        bias_piece(2 * i + 1)
                    for pn, sl in zip(pns, pin_sl):
                        T.add(32 * (2 * p + i + 1) + sl, pn)

        for c_ in [cp_w[1, 1], cp_w[2, 1], cp_wo]:
            c_.wait()
        with scope('unit1'):
            T = Ties(['qkv', 'qkv', 'out'] * NP)
            at = {}
            for p in range(NP):
                for pp in (p, p + 1):
                    if pp < NP and pp not in at:
                        markers, words = attend_steps(RQ0, RK0, RV0, pp)
                        lo = max(96 * pp - u1_back, 14 if pp == 0 else 0)
                        T.spread(markers, lo, 96 * pp - u1_back + u1_len)
                        at[pp] = words
                h = HP[p]
                ms = []
                for i, t in enumerate((1, 2)):
                    m, pns = qdot(h, WQKV, Rset[1][t], p, t, 1, None, T.get(3 * p + i))
                    ms.append(m)
                    for pn, sl in zip(pns, pin_sl):
                        T.add(32 * (3 * p + i + 1) + sl, pn)
                store_o(OS0, p, at[p], zero_of(ms[1]))
                ACC[p] = out_dot(OS0, p, WO, 0, T.get(3 * p + 2))

        for c_ in [cp_w[t, u] for u in (2, 3) for t in range(3)] + cp_xb + [cp_mod2]:
            c_.wait()

        def gemv_piece(i):
            c0 = 128 * i
            g2 = jnp.dot(sc16, WMOD[:, pl.ds(2048 + c0, 128)], preferred_element_type=f32)
            MOD2[:, pl.ds(c0, 128)] = g2[0:8, :]

        carry = []
        with scope('units23'):
          for u in (2, 3):
            Rw = Rset[u % 2]
            Rr = Rset[(u - 1) % 2]
            OS = OSs[(u - 1) % 2]
            with_out = u == 2
            for p in range(NP):
                markers, words = attend_steps(Rr[0], Rr[1], Rr[2], p)
                h = HP[p]
                kinds = ['qkv'] * 3 + (['out'] if with_out else [])
                T = Ties(kinds)
                lt = spread_lhs(markers, 3, at_lo, at_hi if with_out else at3_hi)
                for slot, z in carry:
                    T.add(slot, z)
                carry = []
                order = (0, 1, 2) if with_out else (2, 1, 0)
                ms = []
                for i, t in enumerate(order):
                    m, pns = qdot(h, WQKV, Rw[t], p, t, u, lt.get(i), T.get(i))
                    ms.append(m)
                    if u == 2:
                        gemv_piece(4 * p + i)
                    for pn, sl in zip(pns, pin_sl):
                        tgt = 32 * (i + 1) + sl
                        if not T.add(tgt, pn):
                            carry.append((tgt - 32 * len(kinds), pn))
                store_o(OS, p, words, zero_of(ms[2]) if with_out else None)
                if with_out:
                    ACC[p] += out_dot(OS, p, WO, u - 1, T.get(3))
                    gemv_piece(4 * p + 3)

        ga_t = jnp.tile(MOD2[:, 0:1024], (128 // 8, 1))
        T = Ties(['out'] * 16)
        for slot, z in carry:
            T.add(slot, z)
        at_done = {}
        with scope('t'):
            for d in range(16):
                for p in range(NP):
                    if p not in at_done and (p * t_w) // 32 <= d:
                        markers, words = attend_steps(RQ1, RK1, RV1, p)
                        T.spread(markers, p * t_w + t_lo, p * t_w + t_lo + t_len)
                        at_done[p] = words
                res = out_dot(OS0 if d < 8 else OS1, d % 8, WO, 2 if d < 8 else 3, T.get(d))
                for p in range(NP):
                    endslot = p * t_w + t_lo + t_len
                    if at_done.get(p) is not None and (endslot + t_thr) // 32 <= d:
                        store_o(OS1, p, at_done[p], zero_of(res[0:8, 0:128]))
                        at_done[p] = None
                if d < 8:
                    ACC[d] += res
                else:
                    p = d - 8
                    a = ACC[p] + res
                    lo, hi = unpack2(load_words(XB, p))
                    x1w = pack2(lo + ga_t * a[0:128], hi + ga_t * a[128:256])
                    for j in range(8):
                        X1B[j, pl.ds(p, 128, stride=8), :] = x1w[:, 128 * j:128 * (j + 1)]

        TMF = ffn_tm
        NT = S // TMF
        WR = TMF // 2
        TN = 512

        def ln2_tile(r0w):
            x1 = jnp.concatenate([pltpu.bitcast(X1B[j, pl.ds(r0w, WR), :], bf16) for j in range(8)], axis=1)
            b1 = jnp.tile(1.0 + MOD2[:, 2048:3072], (TMF // 8, 1))
            sb = jnp.tile(MOD2[:, 1024:2048], (TMF // 8, 1))
            return layer_norm(x1.astype(f32)) * b1 + sb

        with scope('ln2_0'):
            H2T[0] = ln2_tile(0).astype(bf16)
        for c_ in cp_ffn:
            c_.wait()

        def ffn_body(r, _):
            w0 = pl.multiple_of(r * WR, WR)
            h = H2T[r % 2]
            wn = pl.multiple_of(jnp.minimum(r + 1, NT - 1) * WR, WR)
            hn = ln2_tile(wn)
            H2T[(r + 1) % 2] = hn.astype(bf16)
            hb = pltpu.bitcast(hn, u32)
            ng = TMF // 16
            pins = [(or_all([hb[16 * g + 8 * i:16 * g + 8 * i + 8, 128 * j:128 * (j + 1)]
                             for i in range(2) for j in range(8)]) >> 31) >> 1 for g in range(ng)]
            acc = None
            for j in range(F // TN):
                hj = h
                if j == 2:
                    hj = tie_lhs(h, {(g, 0): pins[g] for g in range(ng)})
                g = jnp.dot(hj, W1[:, j * TN:(j + 1) * TN], preferred_element_type=f32)
                up = jnp.dot(h, W3[:, j * TN:(j + 1) * TN], preferred_element_type=f32)
                a = (g * jax.nn.sigmoid(g) * up).astype(bf16)
                o = jnp.dot(a, W2[j * TN:(j + 1) * TN, :], preferred_element_type=f32)
                acc = o if acc is None else acc + o
            x1 = jnp.concatenate([pltpu.bitcast(X1B[j, pl.ds(w0, WR), :], bf16) for j in range(8)], axis=1)
            gbt = jnp.tile(MOD2[:, 3072:4096], (TMF // 8, 1))
            out = (x1.astype(f32) + gbt * acc).astype(bf16)
            r0 = pl.multiple_of(r * TMF, TMF)
            OUTB[pl.ds(r0, TMF), :] = out
            pltpu.make_async_copy(OUTB.at[pl.ds(r0, TMF), :], out_hbm.at[0, pl.ds(r0, TMF), :],
                                  sems.at[sem_i[0] + r]).start()
            return 0
        with scope('ffn'):
            lax.fori_loop(0, NT, ffn_body, 0)
        with scope('tail'):
            for r in range(NT):
                pltpu.make_async_copy(OUTB.at[pl.ds(TMF * r, TMF), :], out_hbm.at[0, pl.ds(TMF * r, TMF), :],
                                      sems.at[sem_i[0] + r]).wait()

    return kernel


def build(cfg=None):
    cfg = cfg or {}
    kernel = make_kernel(cfg)
    V = pltpu.VMEM
    scratch = [
        V((1, D), bf16),
        V((8, SPAD, 128), bf16),
        V((8, SPAD, 128), bf16),
        V((4, SPAD, 128), bf16),
        V((4, 128, 128), f32),
        V((NP, TM, D), bf16),
        V((D, 3 * D), bf16),
        V((16, 256, 128), f32), V((32, 256, 128), f32), V((32, 256, 128), f32),
        V((16, 256, 128), f32), V((32, 256, 128), f32), V((32, 256, 128), f32),
        V((NP, 264, 128), u32), V((NP, 264, 128), u32),
        V((D, D), bf16),
        V((NP, TM, D), f32),
        V((2, cfg.get('ffn_tm', 128), D), bf16),
        V((8, WPAD, 128), u32),
        V((D, F), bf16), V((D, F), bf16), V((F, D), bf16),
        V((D, 6 * D), bf16),
        V((S, D), bf16),
        V((8, 2 * D), f32),
        V((8, 4 * D), f32),
        pltpu.SemaphoreType.DMA((64,)),
    ]
    anyspec = pl.BlockSpec(memory_space=pl.ANY)
    return pl.pallas_call(
        kernel,
        out_shape=jax.ShapeDtypeStruct((1, S, D), bf16),
        in_specs=[anyspec] * 8,
        out_specs=anyspec,
        scratch_shapes=scratch,
        compiler_params=pltpu.CompilerParams(vmem_limit_bytes=cfg.get('vmem', 124 * 2 ** 20), flags=cfg.get('flags')),
    )


@jax.jit
def pallas_adaLN_cond__sliding_local_dilated__glu_gated_swiglu__prompt_kernel(
    A_x: jax.Array,
    A_wqkv: jax.Array,
    A_wo: jax.Array,
    B_x: jax.Array,
    B_w1: jax.Array,
    B_w3: jax.Array,
    B_w2: jax.Array,
    c: jax.Array,
    w_mod: jax.Array,
):
    del B_x
    return build({})(A_x, A_wqkv, A_wo, B_w1, B_w3, B_w2, c, w_mod)
```

```python
import contextlib
import functools
import jax
import jax.numpy as jnp
from jax import lax
from jax.experimental import pallas as pl
from jax.experimental.pallas import tpu as pltpu

S, D, F = 2048, 1024, 3584
NP = 8
NU = 4
TM = 256
LOG2E = 1.4426950408889634
QSCALE = (32 ** -0.5) * LOG2E
EPS = 1e-5
SPAD = 2064
WPAD = 1032
f32, bf16, u32 = jnp.float32, jnp.bfloat16, jnp.uint32


def zero_of(v):
    b = pltpu.bitcast(v, u32)
    return (b >> 31) >> 1


def unpack2(w):
    lo = pltpu.unpack_elementwise(w, index=0, packed_dtype=bf16, unpacked_dtype=f32)
    hi = pltpu.unpack_elementwise(w, index=1, packed_dtype=bf16, unpacked_dtype=f32)
    return lo, hi


def pack2(e, o):
    return pltpu.pack_elementwise([e, o], packed_dtype=bf16)


def or_all(vals):
    return functools.reduce(lambda a, b: a | b, vals)


def tie_lhs(h, ties):
    if not ties:
        return h
    K = h.shape[1]
    nk = K // 512 if K >= 512 else 1
    kw = 512 if K >= 512 else K
    rows = []
    for g in range(h.shape[0] // 16):
        blk = h[16 * g:16 * g + 16, :]
        if any((g, kh) in ties for kh in range(nk)):
            cols = []
            for kh in range(nk):
                a = blk[:, kh * kw:(kh + 1) * kw]
                if (g, kh) in ties:
                    a0 = pltpu.bitcast(pltpu.bitcast(a[:, :128], u32) | ties[(g, kh)], bf16)
                    a = jnp.concatenate([a0, a[:, 128:]], axis=1)
                cols.append(a)
            blk = jnp.concatenate(cols, axis=1) if len(cols) > 1 else cols[0]
        rows.append(blk)
    return jnp.concatenate(rows, axis=0)


def tie_rhs(w, ties):
    if not ties:
        return w
    cols = []
    for j in range(w.shape[1] // 128):
        c = w[:, 128 * j:128 * (j + 1)]
        if any(k[1] == j for k in ties):
            rows = []
            for i in range(w.shape[0] // 16):
                b = c[16 * i:16 * i + 16]
                if (i, j) in ties:
                    b = pltpu.bitcast(pltpu.bitcast(b, u32) | ties[(i, j)], bf16)
                rows.append(b)
            c = jnp.concatenate(rows, axis=0)
        cols.append(c)
    return jnp.concatenate(cols, axis=1)


class Ties:
    def __init__(self, kinds):
        self.kinds = kinds
        self.t = [dict() for _ in kinds]
        self.used = {}

    def add(self, g, z):
        g = max(g, 0)
        n = len(self.kinds)
        d, dn = g // 64, (g + 16) // 64
        if dn < n and self.kinds[dn] == 'out':
            d, ts = dn, ((g + 16) % 64) // 2
        elif d < n and self.kinds[d] == 'out':
            ts = 31
        elif d < n:
            cur = self.t[d].get(g % 64)
            self.t[d][g % 64] = z if cur is None else (cur | z)
            return True
        else:
            return False
        k = self.used.get((d, ts), 0)
        self.used[(d, ts)] = k + 1
        k %= 4
        key = (7 - (ts % 8) + 8 * (k // 2), 2 * (ts // 8) + (k % 2))
        cur = self.t[d].get(key)
        self.t[d][key] = z if cur is None else (cur | z)
        return True

    def spread(self, markers, lo, hi):
        n = len(markers)
        for m, mk in enumerate(markers):
            self.add(lo + (m * (hi - lo)) // n, mk)

    def get(self, d):
        return self.t[d]


def dot_k1024(h, w_ref, col, ties):
    ties = ties or {}
    outs = []
    for sub in range(2):
        lt = {((s_ % 16), (s_ % 32) // 16): z for s_, z in ties.items() if s_ // 32 == sub}
        outs.append(jnp.dot(tie_lhs(h, lt), w_ref[:, col + 128 * sub:col + 128 * (sub + 1)], preferred_element_type=f32))
    return jnp.concatenate(outs, axis=1)


def dot_k256(lhs, w_ref, row, ties):
    return jnp.dot(lhs, tie_rhs(w_ref[row:row + 256, :], ties), preferred_element_type=f32)


def ln_stats(x):
    mean = jnp.sum(x, axis=1, keepdims=True) * (1.0 / D)
    xc = x - mean
    var = jnp.sum(xc * xc, axis=1, keepdims=True) * (1.0 / D)
    return xc, lax.rsqrt(var + EPS)


def layer_norm(x):
    xc, r = ln_stats(x)
    return xc * r


def load_words(buf, p):
    return jnp.concatenate([buf.at[j].bitcast(u32)[pl.ds(p, 128, stride=8), :] for j in range(8)], axis=1)


def store_heads(R, idx, j, val):
    for hh in range(4):
        R[idx, pl.ds(4 * j + hh, 32, stride=8), :] = val[32 * hh:32 * hh + 32]


def qdot(h, WQKV, R, p, t, u, ties):
    r = dot_k1024(h, WQKV, t * D + 256 * u, ties)
    marker = r[0:8, 0:128]
    if t == 0:
        r = r * QSCALE
    wd = pack2(r[0:128], r[128:256])
    off = 0 if t == 0 else 16
    pins = []
    for j in range(2):
        wt = wd[:, j * 128:(j + 1) * 128].T
        for hf, val in enumerate(unpack2(wt)):
            store_heads(R, off + 2 * p + hf, j, val)
        if t > 0 and p > 0:
            ws = pltpu.roll(wt, 1, 1)
            for hf, sval in enumerate(unpack2(ws)):
                store_heads(R, 2 * p + hf, j, sval)
            for hh in range(2):
                pins.append((or_all([ws[64 * hh + 8 * i:64 * hh + 8 * i + 8] for i in range(8)]) >> 31) >> 1)
        else:
            pins.append((wt[56:64] >> 31) >> 1)
            pins.append((wt[120:128] >> 31) >> 1)
    return marker, pins


def attend_steps(RQ, RK, RV, p, fine=True):
    lane = lax.broadcasted_iota(jnp.int32, (8, 128), 1)
    markers = []
    Ps = []
    for hf in range(2):
        rho = 2 * p + hf
        q = RQ[rho].reshape(32, 8, 128)
        Ls = []
        for w in range(8):
            kap = rho - 2 * w
            kk = RK[16 + kap].reshape(32, 8, 128)
            qk = q * kk
            ps = [jnp.sum(qk[8 * i:8 * i + 8], axis=0) for i in range(4)]
            L = (ps[0] + ps[1]) + (ps[2] + ps[3])
            if kap < 0:
                L = jnp.where(lane <= 0, -1e9, L)
            Ls.append(L)
            markers.append(zero_of(L))
        m = functools.reduce(jnp.maximum, Ls)
        if fine:
            markers.append(zero_of(m))
        es = [jnp.exp2(L - m) for L in Ls]
        ssum = functools.reduce(jnp.add, es)
        if fine:
            markers.append(zero_of(ssum))
        inv = 1.0 / ssum
        Ps.append([e * inv for e in es])
        markers.append(zero_of(inv))
    words = []
    for dg in range(16):
        ws = []
        for d in range(2 * dg, 2 * dg + 2):
            os_ = []
            for hf in range(2):
                rho = 2 * p + hf
                o = None
                for w in range(8):
                    kap = rho - 2 * w
                    tt = Ps[hf][w] * RV[16 + kap, 8 * d:8 * d + 8, :]
                    o = tt if o is None else o + tt
                os_.append(o)
            ws.append(pack2(os_[0], os_[1]))
        words += ws
        markers.append(zero_of(ws[0] | ws[1]))
    return markers, words


def store_o(OS, p, words, throttle):
    if throttle is not None:
        words = [w | throttle for w in words]
    OS[p, 0:256, :] = jnp.concatenate(words, axis=0)


def out_dot(OS, p, WO, u, rties):
    parts = []
    for jj in range(2):
        rows = [OS[p, pl.ds(4 * jj + hh, 32, stride=8), :] for hh in range(4)]
        parts.append(jnp.concatenate(rows, axis=0).T)
    lo, hi = unpack2(jnp.concatenate(parts, axis=1))
    lhs = jnp.concatenate([lo, hi], axis=0).astype(bf16)
    return dot_k256(lhs, WO, 256 * u, rties)


def make_kernel(cfg):
    pin_sl = cfg.get('pin_sl', (0, 16, 32, 46))
    u1_back, u1_len = cfg.get('u1_back', 56), cfg.get('u1_len', 142)
    ffn_tm = cfg.get('ffn_tm', 128)
    a1_lo, a1_w, a1_len = cfg.get('a1', (4, 256, 140))
    a2_lo, a2_w, a2_len = cfg.get('a2', (2052, 132, 128))
    a3_lo, a3_w, a3_len = cfg.get('a3', (3190, 132, 120))
    thr = cfg.get('thr', 45)
    ln_pins = cfg.get('ln_pins', 16)
    rl0_lo, rl0_hi, rl1_lo, rl1_hi = tuple(cfg.get('rl0', (176, 880))) + tuple(cfg.get('rl1', (24, 1400)))
    nat_lo, nat_hi = cfg.get('nat_lo', 20), cfg.get('nat_hi', 100)

    def scope(name):
        return jax.named_scope(name) if cfg.get('scopes') else contextlib.nullcontext()

    def kernel(x_hbm, wqkv_hbm, wo_hbm, w1_hbm, w3_hbm, w2_hbm, c_hbm, wmod_hbm, out_hbm,
               CV, XB, HB, QN, BQ, HP, WQKV, RQ0, RK0, RV0, RQ1, RK1, RV1, OS0, OS1, WO, ACC, H2T, X1B,
               W1, W3, W2, WMOD, OUTB, MOD1, MOD2, sems):
        Rset = [(RQ0, RK0, RV0), (RQ1, RK1, RV1)]
        OSs = [OS0, OS1]
        XN = OUTB
        sem_i = [0]

        def new_copy(src, dst):
            i = sem_i[0]
            sem_i[0] += 1
            return pltpu.make_async_copy(src, dst, sems.at[i])

        def colcopy(src, dst, c0, n):
            return new_copy(src.at[:, pl.ds(c0, n)], dst.at[:, pl.ds(c0, n)])

        cp_c = new_copy(c_hbm, CV)
        cp_ca = [colcopy(wmod_hbm, WMOD, 1024 + 512 * i, 512) for i in range(2)]
        cp_sa = colcopy(wmod_hbm, WMOD, 0, 1024)
        cp_xn = [new_copy(x_hbm.at[0, pl.ds(TM * r, TM), :], XN.at[pl.ds(TM * r, TM), :]) for r in range(8)]
        cp_w = {(t, u): colcopy(wqkv_hbm, WQKV, t * D + 256 * u, 256) for t in range(3) for u in range(NU)}
        cp_wo = new_copy(wo_hbm, WO)
        cp_xb = [new_copy(x_hbm.at[0, :, pl.ds(128 * j, 128)], XB.at[j, pl.ds(0, S), :]) for j in range(8)]
        cp_mod2 = colcopy(wmod_hbm, WMOD, 2048, 4096)
        cp_ffn = [new_copy(w1_hbm, W1), new_copy(w3_hbm, W3), new_copy(w2_hbm, W2)]

        for c_ in ([cp_c] + cp_ca + [cp_xn[0], cp_w[0, 0], cp_xn[1], cp_w[0, 1]] + cp_xn[2:] + [cp_sa]
                   + [cp_w[1, 0], cp_w[2, 0], cp_w[1, 1], cp_w[2, 1], cp_wo]
                   + [cp_w[t, u] for u in (2, 3) for t in range(3)] + cp_xb + [cp_mod2] + cp_ffn):
            c_.start()

        with scope('mod_ca'):
            cp_c.wait()
            cv = CV[...].astype(f32)
            sc = (cv * jax.nn.sigmoid(cv)).astype(bf16)
            sc16 = jnp.broadcast_to(sc, (16, D))
            for i in range(2):
                cp_ca[i].wait()
                m = jnp.dot(sc16, WMOD[:, 1024 + 512 * i:1024 + 512 * (i + 1)], preferred_element_type=f32)
                MOD1[:, 1024 + 512 * i:1024 + 512 * (i + 1)] = 1.0 + m[0:8]

        def ln_nat(r):
            xc, rs = ln_stats(XN[pl.ds(TM * r, TM), :].astype(f32))
            hm = (xc * rs) * jnp.tile(MOD1[:, 1024:2048], (TM // 8, 1))
            h16 = hm.astype(bf16)
            for j in range(8):
                HB[j, pl.ds(TM * r, TM), :] = h16[:, 128 * j:128 * (j + 1)]
            hb = pltpu.bitcast(hm[:, 896:1024], u32)
            rows = TM // ln_pins
            return [(or_all([hb[rows * g + 8 * i:rows * g + 8 * i + 8] for i in range(rows // 8)]) >> 31) >> 1
                    for g in range(ln_pins)]

        def qnat(r, u, rties):
            hn = jnp.concatenate([HB[j, pl.ds(TM * r, TM), :] for j in range(8)], axis=1)
            res = dot_k1024(hn, WQKV, 256 * u, rties)
            res = (res * QSCALE).astype(bf16)
            for j in range(2):
                QN[2 * u + j, pl.ds(TM * r, TM), :] = res[:, 128 * j:128 * (j + 1)]

        def sa_piece(i):
            m = jnp.dot(sc16, WMOD[:, 128 * i:128 * (i + 1)], preferred_element_type=f32)
            MOD1[:, 128 * i:128 * (i + 1)] = m[0:8]

        with scope('nat0'):
            cp_xn[0].wait()
            ln_nat(0)
            cp_w[0, 0].wait()
            qnat(0, 0, None)
            cp_xn[1].wait()
            ln_nat(1)
            cp_w[0, 1].wait()
            qnat(0, 1, None)

        def nat_region(waits, seq, extra=None):
            for c_ in waits:
                c_.wait()
            T = Ties(['qkv'] * (2 * len(seq)))
            for i, (r, ln_r) in enumerate(seq):
                if ln_r is not None:
                    T.spread(ln_nat(ln_r), 128 * i + nat_lo, 128 * i + nat_hi)
                for k, (rr, u) in enumerate(r):
                    qnat(rr, u, T.get(2 * i + k))
                    if extra:
                        extra(2 * i + k)

        with scope('nat1'):
            nat_region([cp_xn[2]], [([(1, 0), (1, 1)], 2)])
        with scope('nat2'):
            nat_region([cp_xn[3], cp_xn[4]], [([(2, 0), (2, 1)], 3), ([(3, 0), (3, 1)], 4)])
        with scope('nat3'):
            nat_region(cp_xn[5:], [([(4, 0), (4, 1)], 5), ([(5, 0), (5, 1)], 6)])
        with scope('nat4'):
            def sa_extra(d):
                for i in range(2 * d, 2 * d + 2):
                    sa_piece(i)
            nat_region([cp_sa], [([(6, 0), (6, 1)], 7), ([(7, 0), (7, 1)], None)], sa_extra)

        for c_ in [cp_w[1, 0], cp_w[2, 0]]:
            c_.wait()
        sa_t = jnp.tile(MOD1[:, 0:1024], (128 // 8, 1))

        def make_hp(p):
            lo, hi = unpack2(load_words(HB, p))
            h = jnp.concatenate([lo + sa_t, hi + sa_t], axis=0).astype(bf16)
            HP[p] = h
            return h

        def bias_piece(i):
            sa16 = jnp.tile(MOD1[:, 0:1024], (2, 1)).astype(bf16)
            b = jnp.dot(sa16, WQKV[:, 128 * i:128 * (i + 1)], preferred_element_type=f32)[0:8] * QSCALE
            BQ[i] = jnp.tile(b, (16, 1)).T

        def rl_piece(u, j, p):
            w = QN.at[2 * u + j].bitcast(u32)[pl.ds(p, 128, stride=8), :]
            wt = w.T
            last = None
            for hf, val in enumerate(unpack2(wt)):
                val = val + BQ[2 * u + j]
                store_heads(Rset[u][0], 2 * p + hf, j, val)
                last = val
            return (pltpu.bitcast(last[120:128], u32) >> 31) >> 1

        with scope('kv0'):
            T = Ties(['qkv'] * 16)
            pieces = [(0, j, p) for p in range(NP) for j in range(2)]
            for p in range(NP):
                if p == 1:
                    T.spread([rl_piece(*pc) for pc in pieces], rl0_lo, rl0_hi)
                h = make_hp(p)
                for i, t in enumerate((1, 2)):
                    m, pns = qdot(h, WQKV, Rset[0][t], p, t, 0, T.get(2 * p + i))
                    if p == 0:
                        bias_piece(2 * i)
                        bias_piece(2 * i + 1)
                    for pn, sl in zip(pns, pin_sl):
                        T.add(64 * (2 * p + i + 1) + sl, pn)

        for c_ in [cp_w[1, 1], cp_w[2, 1], cp_wo]:
            c_.wait()
        with scope('unit1'):
            T = Ties(['qkv', 'qkv', 'out'] * NP)
            at = {}
            T.spread([rl_piece(1, j, p) for p in range(NP) for j in range(2)], rl1_lo, rl1_hi)
            for p in range(NP):
                for pp in (p, p + 1):
                    if pp < NP and pp not in at:
                        markers, words = attend_steps(RQ0, RK0, RV0, pp)
                        lo = max(192 * pp - u1_back, 8 if pp == 0 else 0)
                        T.spread(markers, lo, 192 * pp - u1_back + u1_len)
                        at[pp] = words
                h = HP[p]
                ms = []
                for i, t in enumerate((1, 2)):
                    m, pns = qdot(h, WQKV, Rset[1][t], p, t, 1, T.get(3 * p + i))
                    ms.append(m)
                    for pn, sl in zip(pns, pin_sl):
                        T.add(64 * (3 * p + i + 1) + sl, pn)
                store_o(OS0, p, at[p], zero_of(ms[1]))
                ACC[p] = out_dot(OS0, p, WO, 0, T.get(3 * p + 2))

        for c_ in [cp_w[t, u] for u in (2, 3) for t in range(3)] + cp_xb + [cp_mod2]:
            c_.wait()

        def gemv_piece(i):
            c0 = 128 * i
            g2 = jnp.dot(sc16, WMOD[:, pl.ds(2048 + c0, 128)], preferred_element_type=f32)
            MOD2[:, pl.ds(c0, 128)] = g2[0:8, :]

        seq = []
        for p in range(NP):
            seq += [('q', 2, 0, p), ('q', 2, 1, p), ('q', 2, 2, p), ('o', 1, p)]
        for p in range(NP):
            seq += [('q', 3, 1, p), ('q', 3, 2, p)]
        seq += [('q', 3, 0, p) for p in range(NP)] + [('o', 2, p) for p in range(NP)] + [('o', 3, p) for p in range(NP)]
        T = Ties(['qkv' if op[0] == 'q' else 'out' for op in seq])
        wins = [(1, p, a1_lo + p * a1_w, a1_lo + p * a1_w + a1_len) for p in range(NP)]
        wins += [(2, p, a2_lo + p * a2_w, a2_lo + p * a2_w + a2_len) for p in range(NP)]
        wins += [(3, p, a3_lo + p * a3_w, a3_lo + p * a3_w + a3_len) for p in range(NP)]
        pend = {}
        with scope('u23t'):
            for d, op in enumerate(seq):
                for (ua, p, lo, hi) in wins:
                    if (ua, p) not in pend and lo // 64 <= d:
                        Ra = Rset[ua % 2]
                        markers, words = attend_steps(Ra[0], Ra[1], Ra[2], p)
                        T.spread(markers, lo, hi)
                        pend[(ua, p)] = words
                if op[0] == 'q':
                    _, u, t, p = op
                    m, pns = qdot(HP[p], WQKV, Rset[u % 2][t], p, t, u, T.get(d))
                    for pn, sl in zip(pns, pin_sl):
                        T.add(64 * (d + 1) + sl, pn)
                else:
                    _, u, p = op
                    assert pend.get((u, p), 0) is None, (u, p)
                    res = out_dot(OSs[u % 2], p, WO, u, T.get(d))
                    m = res[0:8, 0:128]
                if d < 32:
                    gemv_piece(d)
                for (ua, pp, lo, hi) in wins:
                    if pend.get((ua, pp)) is not None and (hi + thr) // 64 <= d:
                        store_o(OSs[ua % 2], pp, pend[(ua, pp)], zero_of(m))
                        pend[(ua, pp)] = None
                if op[0] == 'o':
                    if u < 3:
                        ACC[p] += res
                    else:
                        ga_t = jnp.tile(MOD2[:, 0:1024], (128 // 8, 1))
                        a = ACC[p] + res
                        lo_, hi_ = unpack2(load_words(XB, p))
                        x1w = pack2(lo_ + ga_t * a[0:128], hi_ + ga_t * a[128:256])
                        for j in range(8):
                            X1B[j, pl.ds(p, 128, stride=8), :] = x1w[:, 128 * j:128 * (j + 1)]

        TMF = ffn_tm
        NT = S // TMF
        WR = TMF // 2
        TN = 512

        def ln2_tile(r0w):
            x1 = jnp.concatenate([pltpu.bitcast(X1B[j, pl.ds(r0w, WR), :], bf16) for j in range(8)], axis=1)
            b1 = jnp.tile(1.0 + MOD2[:, 2048:3072], (TMF // 8, 1))
            sb = jnp.tile(MOD2[:, 1024:2048], (TMF // 8, 1))
            return layer_norm(x1.astype(f32)) * b1 + sb

        with scope('ln2_0'):
            H2T[0] = ln2_tile(0).astype(bf16)
        for c_ in cp_ffn:
            c_.wait()

        def ffn_body(r, _):
            w0 = pl.multiple_of(r * WR, WR)
            h = H2T[r % 2]
            wn = pl.multiple_of(jnp.minimum(r + 1, NT - 1) * WR, WR)
            hn = ln2_tile(wn)
            H2T[(r + 1) % 2] = hn.astype(bf16)
            hb = pltpu.bitcast(hn, u32)
            ng = TMF // 16
            pins = [(or_all([hb[16 * g + 8 * i:16 * g + 8 * i + 8, 128 * j:128 * (j + 1)]
                             for i in range(2) for j in range(8)]) >> 31) >> 1 for g in range(ng)]
            acc = None
            for j in range(F // TN):
                hj = h
                if j == 2:
                    hj = tie_lhs(h, {(g, 0): pins[g] for g in range(ng)})
                g = jnp.dot(hj, W1[:, j * TN:(j + 1) * TN], preferred_element_type=f32)
                up = jnp.dot(h, W3[:, j * TN:(j + 1) * TN], preferred_element_type=f32)
                a = (g * jax.nn.sigmoid(g) * up).astype(bf16)
                o = jnp.dot(a, W2[j * TN:(j + 1) * TN, :], preferred_element_type=f32)
                acc = o if acc is None else acc + o
            x1 = jnp.concatenate([pltpu.bitcast(X1B[j, pl.ds(w0, WR), :], bf16) for j in range(8)], axis=1)
            gbt = jnp.tile(MOD2[:, 3072:4096], (TMF // 8, 1))
            out = (x1.astype(f32) + gbt * acc).astype(bf16)
            r0 = pl.multiple_of(r * TMF, TMF)
            OUTB[pl.ds(r0, TMF), :] = out
            pltpu.make_async_copy(OUTB.at[pl.ds(r0, TMF), :], out_hbm.at[0, pl.ds(r0, TMF), :],
                                  sems.at[sem_i[0] + r]).start()
            return 0
        with scope('ffn'):
            lax.fori_loop(0, NT, ffn_body, 0)
        with scope('tail'):
            for r in range(NT):
                pltpu.make_async_copy(OUTB.at[pl.ds(TMF * r, TMF), :], out_hbm.at[0, pl.ds(TMF * r, TMF), :],
                                      sems.at[sem_i[0] + r]).wait()

    return kernel


def build(cfg=None):
    cfg = cfg or {}
    kernel = make_kernel(cfg)
    V = pltpu.VMEM
    scratch = [
        V((1, D), bf16),
        V((8, SPAD, 128), bf16),
        V((8, SPAD, 128), bf16),
        V((4, SPAD, 128), bf16),
        V((4, 128, 128), f32),
        V((NP, TM, D), bf16),
        V((D, 3 * D), bf16),
        V((16, 256, 128), f32), V((32, 256, 128), f32), V((32, 256, 128), f32),
        V((16, 256, 128), f32), V((32, 256, 128), f32), V((32, 256, 128), f32),
        V((NP, 264, 128), u32), V((NP, 264, 128), u32),
        V((D, D), bf16),
        V((NP, TM, D), f32),
        V((2, cfg.get('ffn_tm', 128), D), bf16),
        V((8, WPAD, 128), u32),
        V((D, F), bf16), V((D, F), bf16), V((F, D), bf16),
        V((D, 6 * D), bf16),
        V((S, D), bf16),
        V((8, 2 * D), f32),
        V((8, 4 * D), f32),
        pltpu.SemaphoreType.DMA((64,)),
    ]
    anyspec = pl.BlockSpec(memory_space=pl.ANY)
    return pl.pallas_call(
        kernel,
        out_shape=jax.ShapeDtypeStruct((1, S, D), bf16),
        in_specs=[anyspec] * 8,
        out_specs=anyspec,
        scratch_shapes=scratch,
        compiler_params=pltpu.CompilerParams(vmem_limit_bytes=cfg.get('vmem', 124 * 2 ** 20), flags=cfg.get('flags')),
    )


@jax.jit
def pallas_adaLN_cond__sliding_local_dilated__glu_gated_swiglu__prompt_kernel(
    A_x: jax.Array,
    A_wqkv: jax.Array,
    A_wo: jax.Array,
    B_x: jax.Array,
    B_w1: jax.Array,
    B_w3: jax.Array,
    B_w2: jax.Array,
    c: jax.Array,
    w_mod: jax.Array,
):
    del B_x
    return build({})(A_x, A_wqkv, A_wo, B_w1, B_w3, B_w2, c, w_mod)
```

```python
import contextlib
import functools
import jax
import jax.numpy as jnp
from jax import lax
from jax.experimental import pallas as pl
from jax.experimental.pallas import tpu as pltpu

S, D, F = 2048, 1024, 3584
NP = 8
NU = 4
TM = 256
LOG2E = 1.4426950408889634
QSCALE = (32 ** -0.5) * LOG2E
EPS = 1e-5
SPAD = 2064
WPAD = 1032
f32, bf16, u32 = jnp.float32, jnp.bfloat16, jnp.uint32


def zero_of(v):
    b = pltpu.bitcast(v, u32)
    return (b >> 31) >> 1


def unpack2(w):
    lo = pltpu.unpack_elementwise(w, index=0, packed_dtype=bf16, unpacked_dtype=f32)
    hi = pltpu.unpack_elementwise(w, index=1, packed_dtype=bf16, unpacked_dtype=f32)
    return lo, hi


def pack2(e, o):
    return pltpu.pack_elementwise([e, o], packed_dtype=bf16)


def or_all(vals):
    return functools.reduce(lambda a, b: a | b, vals)


def tie_lhs(h, ties):
    if not ties:
        return h
    K = h.shape[1]
    nk = K // 512 if K >= 512 else 1
    kw = 512 if K >= 512 else K
    rows = []
    for g in range(h.shape[0] // 16):
        blk = h[16 * g:16 * g + 16, :]
        if any((g, kh) in ties for kh in range(nk)):
            cols = []
            for kh in range(nk):
                a = blk[:, kh * kw:(kh + 1) * kw]
                if (g, kh) in ties:
                    a0 = pltpu.bitcast(pltpu.bitcast(a[:, :128], u32) | ties[(g, kh)], bf16)
                    a = jnp.concatenate([a0, a[:, 128:]], axis=1)
                cols.append(a)
            blk = jnp.concatenate(cols, axis=1) if len(cols) > 1 else cols[0]
        rows.append(blk)
    return jnp.concatenate(rows, axis=0)


def tie_rhs(w, ties):
    if not ties:
        return w
    cols = []
    for j in range(w.shape[1] // 128):
        c = w[:, 128 * j:128 * (j + 1)]
        if any(k[1] == j for k in ties):
            rows = []
            for i in range(w.shape[0] // 16):
                b = c[16 * i:16 * i + 16]
                if (i, j) in ties:
                    b = pltpu.bitcast(pltpu.bitcast(b, u32) | ties[(i, j)], bf16)
                rows.append(b)
            c = jnp.concatenate(rows, axis=0)
        cols.append(c)
    return jnp.concatenate(cols, axis=1)


class Ties:
    def __init__(self, kinds):
        self.kinds = kinds
        self.t = [dict() for _ in kinds]
        self.used = {}

    def add(self, g, z):
        g = max(g, 0)
        n = len(self.kinds)
        d, dn = g // 64, (g + 16) // 64
        if dn < n and self.kinds[dn] == 'out':
            d, ts = dn, ((g + 16) % 64) // 2
        elif d < n and self.kinds[d] == 'out':
            ts = 31
        elif d < n:
            cur = self.t[d].get(g % 64)
            self.t[d][g % 64] = z if cur is None else (cur | z)
            return True
        else:
            return False
        k = self.used.get((d, ts), 0)
        self.used[(d, ts)] = k + 1
        k %= 4
        key = (7 - (ts % 8) + 8 * (k // 2), 2 * (ts // 8) + (k % 2))
        cur = self.t[d].get(key)
        self.t[d][key] = z if cur is None else (cur | z)
        return True

    def spread(self, markers, lo, hi):
        n = len(markers)
        for m, mk in enumerate(markers):
            self.add(lo + (m * (hi - lo)) // n, mk)

    def get(self, d):
        return self.t[d]


def dot_k1024(h, w_ref, col, ties):
    ties = ties or {}
    outs = []
    for sub in range(2):
        lt = {((s_ % 16), (s_ % 32) // 16): z for s_, z in ties.items() if s_ // 32 == sub}
        outs.append(jnp.dot(tie_lhs(h, lt), w_ref[:, col + 128 * sub:col + 128 * (sub + 1)], preferred_element_type=f32))
    return jnp.concatenate(outs, axis=1)


def dot_k256(lhs, w_ref, row, ties):
    return jnp.dot(lhs, tie_rhs(w_ref[row:row + 256, :], ties), preferred_element_type=f32)


def ln_stats(x):
    mean = jnp.sum(x, axis=1, keepdims=True) * (1.0 / D)
    xc = x - mean
    var = jnp.sum(xc * xc, axis=1, keepdims=True) * (1.0 / D)
    return xc, lax.rsqrt(var + EPS)


def layer_norm(x):
    xc, r = ln_stats(x)
    return xc * r


def load_words(buf, p):
    return jnp.concatenate([buf.at[j].bitcast(u32)[pl.ds(p, 128, stride=8), :] for j in range(8)], axis=1)


def store_heads(R, idx, j, val):
    for hh in range(4):
        R[idx, pl.ds(4 * j + hh, 32, stride=8), :] = val[32 * hh:32 * hh + 32]


def qdot(h, WQKV, R, p, t, u, ties):
    r = dot_k1024(h, WQKV, t * D + 256 * u, ties)
    marker = r[0:8, 0:128]
    if t == 0:
        r = r * QSCALE
    wd = pack2(r[0:128], r[128:256])
    off = 0 if t == 0 else 16
    pins = []
    for j in range(2):
        wt = wd[:, j * 128:(j + 1) * 128].T
        for hf, val in enumerate(unpack2(wt)):
            store_heads(R, off + 2 * p + hf, j, val)
        if t > 0 and p > 0:
            ws = pltpu.roll(wt, 1, 1)
            for hf, sval in enumerate(unpack2(ws)):
                store_heads(R, 2 * p + hf, j, sval)
            for hh in range(2):
                pins.append((or_all([ws[64 * hh + 8 * i:64 * hh + 8 * i + 8] for i in range(8)]) >> 31) >> 1)
        else:
            pins.append((wt[56:64] >> 31) >> 1)
            pins.append((wt[120:128] >> 31) >> 1)
    return marker, pins


def attend_steps(RQ, RK, RV, p, fine=True):
    lane = lax.broadcasted_iota(jnp.int32, (8, 128), 1)
    markers = []
    Ps = []
    for hf in range(2):
        rho = 2 * p + hf
        q = RQ[rho].reshape(32, 8, 128)
        Ls = []
        for w in range(8):
            kap = rho - 2 * w
            kk = RK[16 + kap].reshape(32, 8, 128)
            qk = q * kk
            ps = [jnp.sum(qk[8 * i:8 * i + 8], axis=0) for i in range(4)]
            L = (ps[0] + ps[1]) + (ps[2] + ps[3])
            if kap < 0:
                L = jnp.where(lane <= 0, -1e9, L)
            Ls.append(L)
            markers.append(zero_of(L))
        m = functools.reduce(jnp.maximum, Ls)
        if fine:
            markers.append(zero_of(m))
        es = [jnp.exp2(L - m) for L in Ls]
        ssum = functools.reduce(jnp.add, es)
        if fine:
            markers.append(zero_of(ssum))
        inv = 1.0 / ssum
        Ps.append([e * inv for e in es])
        markers.append(zero_of(inv))
    words = []
    for dg in range(16):
        ws = []
        for d in range(2 * dg, 2 * dg + 2):
            os_ = []
            for hf in range(2):
                rho = 2 * p + hf
                o = None
                for w in range(8):
                    kap = rho - 2 * w
                    tt = Ps[hf][w] * RV[16 + kap, 8 * d:8 * d + 8, :]
                    o = tt if o is None else o + tt
                os_.append(o)
            ws.append(pack2(os_[0], os_[1]))
        words += ws
        markers.append(zero_of(ws[0] | ws[1]))
    return markers, words


def store_o(OS, p, words, throttle):
    if throttle is not None:
        words = [w | throttle for w in words]
    OS[p, 0:256, :] = jnp.concatenate(words, axis=0)


def out_dot(OS, p, WO, u, rties):
    parts = []
    for jj in range(2):
        rows = [OS[p, pl.ds(4 * jj + hh, 32, stride=8), :] for hh in range(4)]
        parts.append(jnp.concatenate(rows, axis=0).T)
    lo, hi = unpack2(jnp.concatenate(parts, axis=1))
    lhs = jnp.concatenate([lo, hi], axis=0).astype(bf16)
    return dot_k256(lhs, WO, 256 * u, rties)


def make_kernel(cfg):
    pin_sl = cfg.get('pin_sl', (0, 16, 32, 46))
    u1_back, u1_len = cfg.get('u1_back', 56), cfg.get('u1_len', 142)
    ffn_tm = cfg.get('ffn_tm', 128)
    a1_lo, a1_w, a1_len = cfg.get('a1', (4, 256, 140))
    a2_lo, a2_w, a2_len = cfg.get('a2', (2052, 132, 128))
    a3_lo, a3_w, a3_len = cfg.get('a3', (3190, 132, 120))
    thr = cfg.get('thr', 45)
    ln_pins = cfg.get('ln_pins', 16)
    g_mode, g_lo = cfg.get('g_mode', 'vpu'), cfg.get('g_lo', 1)
    rl0_lo, rl0_hi, rl1_lo, rl1_hi = tuple(cfg.get('rl0', (176, 880))) + tuple(cfg.get('rl1', (24, 1400)))
    nat_lo, nat_hi = cfg.get('nat_lo', 20), cfg.get('nat_hi', 100)

    def scope(name):
        return jax.named_scope(name) if cfg.get('scopes') else contextlib.nullcontext()

    def kernel(x_hbm, wqkv_hbm, wo_hbm, w1_hbm, w3_hbm, w2_hbm, c_hbm, wmod_hbm, out_hbm,
               CV, SS, XB, HB, QN, BQ, HP, WQKV, RQ0, RK0, RV0, RQ1, RK1, RV1, OS0, OS1, WO, ACC, H2T, X1B,
               W1, W3, W2, WMOD, OUTB, MOD1, MOD2, sems):
        Rset = [(RQ0, RK0, RV0), (RQ1, RK1, RV1)]
        OSs = [OS0, OS1]
        XN = OUTB
        sem_i = [0]

        def new_copy(src, dst):
            i = sem_i[0]
            sem_i[0] += 1
            return pltpu.make_async_copy(src, dst, sems.at[i])

        def colcopy(src, dst, c0, n):
            return new_copy(src.at[:, pl.ds(c0, n)], dst.at[:, pl.ds(c0, n)])

        cp_c = new_copy(c_hbm, CV)
        cp_ca = [colcopy(wmod_hbm, WMOD, 1024 + 512 * i, 512) for i in range(2)]
        cp_sa = colcopy(wmod_hbm, WMOD, 0, 1024)
        cp_xn = [new_copy(x_hbm.at[0, pl.ds(TM * r, TM), :], XN.at[pl.ds(TM * r, TM), :]) for r in range(8)]
        cp_w = {(t, u): colcopy(wqkv_hbm, WQKV, t * D + 256 * u, 256) for t in range(3) for u in range(NU)}
        cp_wo = new_copy(wo_hbm, WO)
        cp_xb = [new_copy(x_hbm.at[0, :, pl.ds(128 * j, 128)], XB.at[j, pl.ds(0, S), :]) for j in range(8)]
        cp_mod2 = colcopy(wmod_hbm, WMOD, 2048, 4096)
        TH = F // 2
        cp_ffn = []
        for k_ in range(2):
            cp_ffn += [new_copy(w1_hbm.at[:, pl.ds(k_ * TH, TH)], W1.at[k_]),
                       new_copy(w3_hbm.at[:, pl.ds(k_ * TH, TH)], W3.at[k_]),
                       new_copy(w2_hbm.at[pl.ds(k_ * TH, TH), :], W2.at[k_])]

        for c_ in ([cp_c] + cp_ca + [cp_xn[0], cp_w[0, 0], cp_w[0, 1]] + cp_xn[1:] + [cp_sa]
                   + [cp_w[1, 0], cp_w[2, 0], cp_w[1, 1], cp_w[2, 1], cp_wo]
                   + [cp_w[t, u] for u in (2, 3) for t in range(3)] + cp_xb + [cp_mod2] + cp_ffn):
            c_.start()

        with scope('mod_ca'):
            with scope('w_c'):
                cp_c.wait()
            cv = CV[...].astype(f32)
            sc = (cv * jax.nn.sigmoid(cv)).astype(bf16)
            sc16 = jnp.broadcast_to(sc, (16, D))
            SS[...] = jnp.broadcast_to(sc.astype(f32), (128, D)).T
            for i in range(2):
                with scope(f'w_ca{i}'):
                    cp_ca[i].wait()
                m = jnp.dot(sc16, WMOD[:, 1024 + 512 * i:1024 + 512 * (i + 1)], preferred_element_type=f32)
                MOD1[:, 1024 + 512 * i:1024 + 512 * (i + 1)] = 1.0 + m[0:8]

        def ln_nat(r):
            xc, rs = ln_stats(XN[pl.ds(TM * r, TM), :].astype(f32))
            hm = (xc * rs) * jnp.tile(MOD1[:, 1024:2048], (TM // 8, 1))
            h16 = hm.astype(bf16)
            for j in range(8):
                HB[j, pl.ds(TM * r, TM), :] = h16[:, 128 * j:128 * (j + 1)]
            hb = pltpu.bitcast(hm[:, 896:1024], u32)
            rows = TM // ln_pins
            return [(or_all([hb[rows * g + 8 * i:rows * g + 8 * i + 8] for i in range(rows // 8)]) >> 31) >> 1
                    for g in range(ln_pins)]

        def qnat(r, u, rties):
            hn = jnp.concatenate([HB[j, pl.ds(TM * r, TM), :] for j in range(8)], axis=1)
            res = dot_k1024(hn, WQKV, 256 * u, rties)
            res = (res * QSCALE).astype(bf16)
            for j in range(2):
                QN[2 * u + j, pl.ds(TM * r, TM), :] = res[:, 128 * j:128 * (j + 1)]

        def sa_piece(i):
            m = jnp.dot(sc16, WMOD[:, 128 * i:128 * (i + 1)], preferred_element_type=f32)
            MOD1[:, 128 * i:128 * (i + 1)] = m[0:8]

        with scope('nat0'):
            with scope('w_x0'):
                cp_xn[0].wait()
            ln_nat(0)
            with scope('w_q0'):
                cp_w[0, 0].wait()
            qnat(0, 0, None)
            with scope('w_q1'):
                cp_w[0, 1].wait()
            qnat(0, 1, None)
            with scope('w_x1'):
                cp_xn[1].wait()
            ln_nat(1)

        def nat_region(waits, seq, extra=None):
            for c_ in waits:
                c_.wait()
            T = Ties(['qkv'] * (2 * len(seq)))
            for i, (r, ln_r) in enumerate(seq):
                if ln_r is not None:
                    T.spread(ln_nat(ln_r), 128 * i + nat_lo, 128 * i + nat_hi)
                for k, (rr, u) in enumerate(r):
                    qnat(rr, u, T.get(2 * i + k))
                    if extra:
                        extra(2 * i + k)

        with scope('nat1'):
            nat_region([cp_xn[2]], [([(1, 0), (1, 1)], 2)])
        with scope('nat2'):
            nat_region([cp_xn[3], cp_xn[4]], [([(2, 0), (2, 1)], 3), ([(3, 0), (3, 1)], 4)])
        with scope('nat3'):
            nat_region(cp_xn[5:], [([(4, 0), (4, 1)], 5), ([(5, 0), (5, 1)], 6)])
        with scope('nat4'):
            def sa_extra(d):
                for i in range(2 * d, 2 * d + 2):
                    sa_piece(i)
            nat_region([cp_sa], [([(6, 0), (6, 1)], 7), ([(7, 0), (7, 1)], None)], sa_extra)

        for c_ in [cp_w[1, 0], cp_w[2, 0]]:
            c_.wait()
        sa_t = jnp.tile(MOD1[:, 0:1024], (128 // 8, 1))

        def make_hp(p):
            lo, hi = unpack2(load_words(HB, p))
            h = jnp.concatenate([lo + sa_t, hi + sa_t], axis=0).astype(bf16)
            HP[p] = h
            return h

        def bias_piece(i):
            sa16 = jnp.tile(MOD1[:, 0:1024], (2, 1)).astype(bf16)
            b = jnp.dot(sa16, WQKV[:, 128 * i:128 * (i + 1)], preferred_element_type=f32)[0:8] * QSCALE
            BQ[i] = jnp.tile(b, (16, 1)).T

        def rl_piece(u, j, p):
            w = QN.at[2 * u + j].bitcast(u32)[pl.ds(p, 128, stride=8), :]
            wt = w.T
            last = None
            for hf, val in enumerate(unpack2(wt)):
                val = val + BQ[2 * u + j]
                store_heads(Rset[u][0], 2 * p + hf, j, val)
                last = val
            return (pltpu.bitcast(last[120:128], u32) >> 31) >> 1

        with scope('kv0'):
            T = Ties(['qkv'] * 16)
            pieces = [(0, j, p) for p in range(NP) for j in range(2)]
            for p in range(NP):
                if p == 1:
                    T.spread([rl_piece(*pc) for pc in pieces], rl0_lo, rl0_hi)
                h = make_hp(p)
                for i, t in enumerate((1, 2)):
                    m, pns = qdot(h, WQKV, Rset[0][t], p, t, 0, T.get(2 * p + i))
                    if p == 0:
                        bias_piece(2 * i)
                        bias_piece(2 * i + 1)
                    for pn, sl in zip(pns, pin_sl):
                        T.add(64 * (2 * p + i + 1) + sl, pn)

        for c_ in [cp_w[1, 1], cp_w[2, 1], cp_wo]:
            c_.wait()
        with scope('unit1'):
            T = Ties(['qkv', 'qkv', 'out'] * NP)
            at = {}
            T.spread([rl_piece(1, j, p) for p in range(NP) for j in range(2)], rl1_lo, rl1_hi)
            for p in range(NP):
                for pp in (p, p + 1):
                    if pp < NP and pp not in at:
                        markers, words = attend_steps(RQ0, RK0, RV0, pp)
                        lo = max(192 * pp - u1_back, 8 if pp == 0 else 0)
                        T.spread(markers, lo, 192 * pp - u1_back + u1_len)
                        at[pp] = words
                h = HP[p]
                ms = []
                for i, t in enumerate((1, 2)):
                    m, pns = qdot(h, WQKV, Rset[1][t], p, t, 1, T.get(3 * p + i))
                    ms.append(m)
                    for pn, sl in zip(pns, pin_sl):
                        T.add(64 * (3 * p + i + 1) + sl, pn)
                store_o(OS0, p, at[p], zero_of(ms[1]))
                ACC[p] = out_dot(OS0, p, WO, 0, T.get(3 * p + 2))

        for c_ in [cp_w[t, u] for u in (2, 3) for t in range(3)] + cp_xb + [cp_mod2]:
            c_.wait()

        def vgemv(i):
            c0 = 2048 + 128 * i
            acc = None
            marks = []
            for g in range(64):
                w = WMOD[16 * g:16 * g + 16, c0:c0 + 128].astype(f32) * SS[16 * g:16 * g + 16, :]
                t = w[0:8] + w[8:16]
                acc = t if acc is None else acc + t
                if g % 16 == 15:
                    marks.append(zero_of(acc))
            MOD2[:, 128 * i:128 * (i + 1)] = jnp.broadcast_to(jnp.sum(acc, axis=0, keepdims=True), (8, 128))
            return marks

        def gemv_piece(i):
            c0 = 128 * i
            g2 = jnp.dot(sc16, WMOD[:, pl.ds(2048 + c0, 128)], preferred_element_type=f32)
            MOD2[:, pl.ds(c0, 128)] = g2[0:8, :]

        seq = []
        for p in range(NP):
            seq += [('q', 2, 0, p), ('q', 2, 1, p), ('q', 2, 2, p), ('o', 1, p)]
        for p in range(NP):
            seq += [('q', 3, 1, p), ('q', 3, 2, p)]
        seq += [('q', 3, 0, p) for p in range(NP)] + [('o', 2, p) for p in range(NP)] + [('o', 3, p) for p in range(NP)]
        T = Ties(['qkv' if op[0] == 'q' else 'out' for op in seq])
        wins = [(1, p, a1_lo + p * a1_w, a1_lo + p * a1_w + a1_len) for p in range(NP)]
        wins += [(2, p, a2_lo + p * a2_w, a2_lo + p * a2_w + a2_len) for p in range(NP)]
        wins += [(3, p, a3_lo + p * a3_w, a3_lo + p * a3_w + a3_len) for p in range(NP)]
        pend = {}
        with scope('u23t'):
            for d, op in enumerate(seq):
                for (ua, p, lo, hi) in wins:
                    if (ua, p) not in pend and lo // 64 <= d:
                        Ra = Rset[ua % 2]
                        markers, words = attend_steps(Ra[0], Ra[1], Ra[2], p)
                        T.spread(markers, lo, hi)
                        pend[(ua, p)] = words
                if op[0] == 'q':
                    _, u, t, p = op
                    m, pns = qdot(HP[p], WQKV, Rset[u % 2][t], p, t, u, T.get(d))
                    for pn, sl in zip(pns, pin_sl):
                        T.add(64 * (d + 1) + sl, pn)
                else:
                    _, u, p = op
                    assert pend.get((u, p), 0) is None, (u, p)
                    res = out_dot(OSs[u % 2], p, WO, u, T.get(d))
                    m = res[0:8, 0:128]
                if g_mode == 'mxu':
                    if d < 32:
                        gemv_piece(d)
                elif g_lo <= d + 1 < g_lo + 32:
                    T.spread(vgemv(d + 1 - g_lo), 64 * (d + 1) + 6, 64 * (d + 1) + 64)
                for (ua, pp, lo, hi) in wins:
                    if pend.get((ua, pp)) is not None and (hi + thr) // 64 <= d:
                        store_o(OSs[ua % 2], pp, pend[(ua, pp)], zero_of(m))
                        pend[(ua, pp)] = None
                if op[0] == 'o':
                    if u < 3:
                        ACC[p] += res
                    else:
                        ga_t = jnp.tile(MOD2[:, 0:1024], (128 // 8, 1))
                        a = ACC[p] + res
                        lo_, hi_ = unpack2(load_words(XB, p))
                        x1w = pack2(lo_ + ga_t * a[0:128], hi_ + ga_t * a[128:256])
                        for j in range(8):
                            X1B[j, pl.ds(p, 128, stride=8), :] = x1w[:, 128 * j:128 * (j + 1)]

        TC = 256

        def ln2_rows(r0w):
            x1 = jnp.concatenate([pltpu.bitcast(X1B[j, pl.ds(r0w, 64), :], bf16) for j in range(8)], axis=1)
            b1 = jnp.tile(1.0 + MOD2[:, 2048:3072], (128 // 8, 1))
            sb = jnp.tile(MOD2[:, 1024:2048], (128 // 8, 1))
            return layer_norm(x1.astype(f32)) * b1 + sb

        def epilogue(rp, k):
            w0 = pl.multiple_of(rp * 128 + k * 64, 64)
            x1 = jnp.concatenate([pltpu.bitcast(X1B[j, pl.ds(w0, 64), :], bf16) for j in range(8)], axis=1)
            gbt = jnp.tile(MOD2[:, 3072:4096], (128 // 8, 1))
            a0 = pl.multiple_of(k * 128, 128)
            out = x1.astype(f32) + gbt * ACC[rp % 2, pl.ds(a0, 128), :]
            r0 = pl.multiple_of(rp * 256 + k * 128, 128)
            OUTB[pl.ds(r0, 128), :] = out.astype(bf16)
            return out

        def out_copy(i):
            r0 = i * 128 if isinstance(i, int) else pl.multiple_of(i * 128, 128)
            return pltpu.make_async_copy(OUTB.at[pl.ds(r0, 128), :], out_hbm.at[0, pl.ds(r0, 128), :],
                                         sems.at[sem_i[0] + i])

        def pins_of(v):
            b = pltpu.bitcast(v, u32)
            return [(or_all([b[16 * g + 8 * i:16 * g + 8 * i + 8, 128 * j:128 * (j + 1)]
                             for i in range(2) for j in range(8)]) >> 31) >> 1 for g in range(8)]

        with scope('ln2_0'):
            H2T[0, 0:128, :] = ln2_rows(0).astype(bf16)
            H2T[0, 128:256, :] = ln2_rows(64).astype(bf16)
        for c_ in cp_ffn:
            c_.wait()

        def ffn_body(i, _):
            r = i // 2
            k = i % 2
            h = H2T[r % 2]
            hn = ln2_rows(pl.multiple_of(jnp.minimum(r + 1, 7) * 128 + k * 64, 64))
            H2T[(r + 1) % 2, pl.ds(pl.multiple_of(k * 128, 128), 128), :] = hn.astype(bf16)
            pa = pins_of(hn)
            pb = pins_of(epilogue(jnp.maximum(r - 1, 0), k))
            acc = None
            for j in range(TH // TC):
                sel = {}
                for g in range(8):
                    if 1 + g // 2 == j:
                        sel[(4 * (g % 2), 0)] = pa[g]
                    if 2 + g // 2 == j:
                        sel[(4 * (g % 2) + 8, 0)] = pb[g]
                cs = pl.ds(j * TC, TC)
                g_ = jnp.dot(tie_lhs(h, sel), W1[k, :, cs], preferred_element_type=f32)
                up = jnp.dot(h, W3[k, :, cs], preferred_element_type=f32)
                a = (g_ * jax.nn.sigmoid(g_) * up).astype(bf16)
                o = jnp.dot(a, W2[k, cs, :], preferred_element_type=f32)
                acc = o if acc is None else acc + o
            ACC[r % 2] = acc + jnp.where(k == 0, 0.0, ACC[r % 2])

            @pl.when(i >= 2)
            def _():
                out_copy(i - 2).start()
            return 0
        with scope('ffn'):
            lax.fori_loop(0, 16, ffn_body, 0)
        with scope('tail'):
            epilogue(7, 0)
            out_copy(14).start()
            epilogue(7, 1)
            out_copy(15).start()
            for i in range(16):
                out_copy(i).wait()

    return kernel


def build(cfg=None):
    cfg = cfg or {}
    kernel = make_kernel(cfg)
    V = pltpu.VMEM
    scratch = [
        V((1, D), bf16),
        V((D, 128), f32),
        V((8, SPAD, 128), bf16),
        V((8, SPAD, 128), bf16),
        V((4, SPAD, 128), bf16),
        V((4, 128, 128), f32),
        V((NP, TM, D), bf16),
        V((D, 3 * D), bf16),
        V((16, 256, 128), f32), V((32, 256, 128), f32), V((32, 256, 128), f32),
        V((16, 256, 128), f32), V((32, 256, 128), f32), V((32, 256, 128), f32),
        V((NP, 264, 128), u32), V((NP, 264, 128), u32),
        V((D, D), bf16),
        V((NP, TM, D), f32),
        V((2, TM, D), bf16),
        V((8, WPAD, 128), u32),
        V((2, D, F // 2), bf16), V((2, D, F // 2), bf16), V((2, F // 2, D), bf16),
        V((D, 6 * D), bf16),
        V((S, D), bf16),
        V((8, 2 * D), f32),
        V((8, 4 * D), f32),
        pltpu.SemaphoreType.DMA((64,)),
    ]
    anyspec = pl.BlockSpec(memory_space=pl.ANY)
    return pl.pallas_call(
        kernel,
        out_shape=jax.ShapeDtypeStruct((1, S, D), bf16),
        in_specs=[anyspec] * 8,
        out_specs=anyspec,
        scratch_shapes=scratch,
        compiler_params=pltpu.CompilerParams(vmem_limit_bytes=cfg.get('vmem', 124 * 2 ** 20), flags=cfg.get('flags')),
    )


@jax.jit
def pallas_adaLN_cond__sliding_local_dilated__glu_gated_swiglu__prompt_kernel(
    A_x: jax.Array,
    A_wqkv: jax.Array,
    A_wo: jax.Array,
    B_x: jax.Array,
    B_w1: jax.Array,
    B_w3: jax.Array,
    B_w2: jax.Array,
    c: jax.Array,
    w_mod: jax.Array,
):
    del B_x
    return build({})(A_x, A_wqkv, A_wo, B_w1, B_w3, B_w2, c, w_mod)
```

```python
import contextlib
import functools
import jax
import jax.numpy as jnp
from jax import lax
from jax.experimental import pallas as pl
from jax.experimental.pallas import tpu as pltpu

S, D, F = 2048, 1024, 3584
NP = 8
NU = 4
TM = 256
LOG2E = 1.4426950408889634
QSCALE = (32 ** -0.5) * LOG2E
EPS = 1e-5
SPAD = 2064
WPAD = 1032
f32, bf16, u32 = jnp.float32, jnp.bfloat16, jnp.uint32


def zero_of(v):
    b = pltpu.bitcast(v, u32)
    return (b >> 31) >> 1


def unpack2(w):
    lo = pltpu.unpack_elementwise(w, index=0, packed_dtype=bf16, unpacked_dtype=f32)
    hi = pltpu.unpack_elementwise(w, index=1, packed_dtype=bf16, unpacked_dtype=f32)
    return lo, hi


def pack2(e, o):
    return pltpu.pack_elementwise([e, o], packed_dtype=bf16)


def or_all(vals):
    return functools.reduce(lambda a, b: a | b, vals)


def tie_lhs(h, ties):
    if not ties:
        return h
    K = h.shape[1]
    nk = K // 512 if K >= 512 else 1
    kw = 512 if K >= 512 else K
    rows = []
    for g in range(h.shape[0] // 16):
        blk = h[16 * g:16 * g + 16, :]
        if any((g, kh) in ties for kh in range(nk)):
            cols = []
            for kh in range(nk):
                a = blk[:, kh * kw:(kh + 1) * kw]
                if (g, kh) in ties:
                    a0 = pltpu.bitcast(pltpu.bitcast(a[:, :128], u32) | ties[(g, kh)], bf16)
                    a = jnp.concatenate([a0, a[:, 128:]], axis=1)
                cols.append(a)
            blk = jnp.concatenate(cols, axis=1) if len(cols) > 1 else cols[0]
        rows.append(blk)
    return jnp.concatenate(rows, axis=0)


def tie_rhs(w, ties):
    if not ties:
        return w
    cols = []
    for j in range(w.shape[1] // 128):
        c = w[:, 128 * j:128 * (j + 1)]
        if any(k[1] == j for k in ties):
            rows = []
            for i in range(w.shape[0] // 16):
                b = c[16 * i:16 * i + 16]
                if (i, j) in ties:
                    b = pltpu.bitcast(pltpu.bitcast(b, u32) | ties[(i, j)], bf16)
                rows.append(b)
            c = jnp.concatenate(rows, axis=0)
        cols.append(c)
    return jnp.concatenate(cols, axis=1)


class Ties:
    def __init__(self, kinds):
        self.kinds = kinds
        self.t = [dict() for _ in kinds]
        self.used = {}

    def add(self, g, z):
        g = max(g, 0)
        n = len(self.kinds)
        d, dn = g // 64, (g + 16) // 64
        if dn < n and self.kinds[dn] == 'out':
            d, ts = dn, ((g + 16) % 64) // 2
        elif d < n and self.kinds[d] == 'out':
            ts = 31
        elif d < n:
            cur = self.t[d].get(g % 64)
            self.t[d][g % 64] = z if cur is None else (cur | z)
            return True
        else:
            return False
        k = self.used.get((d, ts), 0)
        self.used[(d, ts)] = k + 1
        k %= 4
        key = (7 - (ts % 8) + 8 * (k // 2), 2 * (ts // 8) + (k % 2))
        cur = self.t[d].get(key)
        self.t[d][key] = z if cur is None else (cur | z)
        return True

    def spread(self, markers, lo, hi):
        n = len(markers)
        for m, mk in enumerate(markers):
            self.add(lo + (m * (hi - lo)) // n, mk)

    def get(self, d):
        return self.t[d]


def dot_k1024(h, w_ref, col, ties):
    ties = ties or {}
    outs = []
    for sub in range(2):
        lt = {((s_ % 16), (s_ % 32) // 16): z for s_, z in ties.items() if s_ // 32 == sub}
        outs.append(jnp.dot(tie_lhs(h, lt), w_ref[:, col + 128 * sub:col + 128 * (sub + 1)], preferred_element_type=f32))
    return jnp.concatenate(outs, axis=1)


def dot_k256(lhs, w_ref, row, ties):
    return jnp.dot(lhs, tie_rhs(w_ref[row:row + 256, :], ties), preferred_element_type=f32)


def ln_stats(x):
    mean = jnp.sum(x, axis=1, keepdims=True) * (1.0 / D)
    xc = x - mean
    var = jnp.sum(xc * xc, axis=1, keepdims=True) * (1.0 / D)
    return xc, lax.rsqrt(var + EPS)


def layer_norm(x):
    xc, r = ln_stats(x)
    return xc * r


def load_words(buf, p):
    return jnp.concatenate([buf.at[j].bitcast(u32)[pl.ds(p, 128, stride=8), :] for j in range(8)], axis=1)


def store_heads(R, idx, j, val):
    for hh in range(4):
        R[idx, pl.ds(4 * j + hh, 32, stride=8), :] = val[32 * hh:32 * hh + 32]


def qdot(h, WQKV, R, p, t, u, ties):
    r = dot_k1024(h, WQKV, t * D + 256 * u, ties)
    marker = r[0:8, 0:128]
    if t == 0:
        r = r * QSCALE
    wd = pack2(r[0:128], r[128:256])
    off = 0 if t == 0 else 16
    pins = []
    for j in range(2):
        wt = wd[:, j * 128:(j + 1) * 128].T
        for hf, val in enumerate(unpack2(wt)):
            store_heads(R, off + 2 * p + hf, j, val)
        if t > 0 and p > 0:
            ws = pltpu.roll(wt, 1, 1)
            for hf, sval in enumerate(unpack2(ws)):
                store_heads(R, 2 * p + hf, j, sval)
            for hh in range(2):
                pins.append((or_all([ws[64 * hh + 8 * i:64 * hh + 8 * i + 8] for i in range(8)]) >> 31) >> 1)
        else:
            pins.append((wt[56:64] >> 31) >> 1)
            pins.append((wt[120:128] >> 31) >> 1)
    return marker, pins


def attend_steps(RQ, RK, RV, p, fine=True):
    lane = lax.broadcasted_iota(jnp.int32, (8, 128), 1)
    markers = []
    Ps = []
    for hf in range(2):
        rho = 2 * p + hf
        q = RQ[rho, 0:256, :].reshape(32, 8, 128)
        Ls = []
        for w in range(8):
            kap = rho - 2 * w
            kk = RK[16 + kap, 0:256, :].reshape(32, 8, 128)
            qk = q * kk
            ps = [jnp.sum(qk[8 * i:8 * i + 8], axis=0) for i in range(4)]
            L = (ps[0] + ps[1]) + (ps[2] + ps[3])
            if kap < 0:
                L = jnp.where(lane <= 0, -1e9, L)
            Ls.append(L)
            markers.append(zero_of(L))
        m = functools.reduce(jnp.maximum, Ls)
        if fine:
            markers.append(zero_of(m))
        es = [jnp.exp2(L - m) for L in Ls]
        ssum = functools.reduce(jnp.add, es)
        if fine:
            markers.append(zero_of(ssum))
        inv = 1.0 / ssum
        Ps.append([e * inv for e in es])
        markers.append(zero_of(inv))
    words = []
    for dg in range(16):
        ws = []
        for d in range(2 * dg, 2 * dg + 2):
            os_ = []
            for hf in range(2):
                rho = 2 * p + hf
                o = None
                for w in range(8):
                    kap = rho - 2 * w
                    tt = Ps[hf][w] * RV[16 + kap, 8 * d:8 * d + 8, :]
                    o = tt if o is None else o + tt
                os_.append(o)
            ws.append(pack2(os_[0], os_[1]))
        words += ws
        markers.append(zero_of(ws[0] | ws[1]))
    return markers, words


def store_o(OS, p, words, throttle):
    if throttle is not None:
        words = [w | throttle for w in words]
    low = lax.broadcasted_iota(jnp.int32, (8, 128), 0) < 4
    a, b = [], []
    for i in range(16):
        x0, x1 = words[2 * i], words[2 * i + 1]
        a.append(jnp.where(low, x0, pltpu.roll(x1, 4, 0)))
        b.append(jnp.where(low, pltpu.roll(x0, 4, 0), x1))
    OS[p, 0:128, :] = jnp.concatenate(a, axis=0)
    OS[p, 136:264, :] = jnp.concatenate(b, axis=0)


def out_dot(OS, p, WO, u, rties):
    parts = []
    for jj in range(2):
        rows = [OS[p, pl.ds(136 * jj + hh, 32, stride=4), :] for hh in range(4)]
        parts.append(jnp.concatenate(rows, axis=0).T)
    lo, hi = unpack2(jnp.concatenate(parts, axis=1))
    lhs = jnp.concatenate([lo, hi], axis=0).astype(bf16)
    return dot_k256(lhs, WO, 256 * u, rties)


def make_kernel(cfg):
    pin_sl = cfg.get('pin_sl', (0, 16, 32, 46))
    u1_back, u1_len = cfg.get('u1_back', 56), cfg.get('u1_len', 142)
    ffn_tm = cfg.get('ffn_tm', 128)
    a1_lo, a1_w, a1_len = cfg.get('a1', (4, 256, 140))
    a2_lo, a2_w, a2_len = cfg.get('a2', (2052, 132, 128))
    a3_lo, a3_w, a3_len = cfg.get('a3', (3190, 132, 120))
    thr = cfg.get('thr', 45)
    ln_pins = cfg.get('ln_pins', 16)
    g_mode, g_lo = cfg.get('g_mode', 'vpu'), cfg.get('g_lo', 1)
    rl0_lo, rl0_hi, rl1_lo, rl1_hi = tuple(cfg.get('rl0', (176, 880))) + tuple(cfg.get('rl1', (24, 1400)))
    nat_lo, nat_hi = cfg.get('nat_lo', 20), cfg.get('nat_hi', 100)

    def scope(name):
        return jax.named_scope(name) if cfg.get('scopes') else contextlib.nullcontext()

    def kernel(x_hbm, wqkv_hbm, wo_hbm, w1_hbm, w3_hbm, w2_hbm, c_hbm, wmod_hbm, out_hbm,
               CV, SS, HB, QN, BQ, HP, WQKV, RQ0, RK0, RV0, RQ1, RK1, RV1, OS0, OS1, WO, ACC, H2T, X1B,
               W1, W3, W2, WMOD, OUTB, MOD1, MOD2, sems):
        Rset = [(RQ0, RK0, RV0), (RQ1, RK1, RV1)]
        OSs = [OS0, OS1]
        XN = OUTB
        sem_i = [0]

        def new_copy(src, dst):
            i = sem_i[0]
            sem_i[0] += 1
            return pltpu.make_async_copy(src, dst, sems.at[i])

        def colcopy(src, dst, c0, n):
            return new_copy(src.at[:, pl.ds(c0, n)], dst.at[:, pl.ds(c0, n)])

        cp_c = new_copy(c_hbm, CV)
        cp_ca = [colcopy(wmod_hbm, WMOD, 1024 + 512 * i, 512) for i in range(2)]
        cp_sa = colcopy(wmod_hbm, WMOD, 0, 1024)
        cp_xn = [new_copy(x_hbm.at[0, pl.ds(TM * r, TM), :], XN.at[pl.ds(TM * r, TM), :]) for r in range(8)]
        cp_w = {(t, u): colcopy(wqkv_hbm, WQKV, t * D + 256 * u, 256) for t in range(3) for u in range(NU)}
        cp_wo = new_copy(wo_hbm, WO)
        cp_mod2 = colcopy(wmod_hbm, WMOD, 2048, 4096)
        TH = F // 2
        cp_ffn = []
        for k_ in range(2):
            cp_ffn += [new_copy(w1_hbm.at[:, pl.ds(k_ * TH, TH)], W1.at[k_]),
                       new_copy(w3_hbm.at[:, pl.ds(k_ * TH, TH)], W3.at[k_]),
                       new_copy(w2_hbm.at[pl.ds(k_ * TH, TH), :], W2.at[k_])]

        for c_ in ([cp_c] + cp_ca + [cp_xn[0], cp_w[0, 0], cp_w[0, 1]] + cp_xn[1:] + [cp_sa]
                   + [cp_w[1, 0], cp_w[2, 0], cp_w[1, 1], cp_w[2, 1], cp_wo]
                   + [cp_w[t, u] for u in (2, 3) for t in range(3)] + [cp_mod2] + cp_ffn):
            c_.start()

        with scope('mod_ca'):
            with scope('w_c'):
                cp_c.wait()
            cv = CV[...].astype(f32)
            sc = (cv * jax.nn.sigmoid(cv)).astype(bf16)
            sc16 = jnp.broadcast_to(sc, (16, D))
            SS[...] = jnp.broadcast_to(sc.astype(f32), (128, D)).T
            for i in range(2):
                with scope(f'w_ca{i}'):
                    cp_ca[i].wait()
                m = jnp.dot(sc16, WMOD[:, 1024 + 512 * i:1024 + 512 * (i + 1)], preferred_element_type=f32)
                MOD1[:, 1024 + 512 * i:1024 + 512 * (i + 1)] = 1.0 + m[0:8]

        def ln_nat(r):
            xc, rs = ln_stats(XN[pl.ds(TM * r, TM), :].astype(f32))
            hm = (xc * rs) * jnp.tile(MOD1[:, 1024:2048], (TM // 8, 1))
            h16 = hm.astype(bf16)
            for j in range(8):
                HB[j, pl.ds(TM * r, TM), :] = h16[:, 128 * j:128 * (j + 1)]
            hb = pltpu.bitcast(hm[:, 896:1024], u32)
            rows = TM // ln_pins
            return [(or_all([hb[rows * g + 8 * i:rows * g + 8 * i + 8] for i in range(rows // 8)]) >> 31) >> 1
                    for g in range(ln_pins)]

        def qnat(r, u, rties):
            hn = jnp.concatenate([HB[j, pl.ds(TM * r, TM), :] for j in range(8)], axis=1)
            res = dot_k1024(hn, WQKV, 256 * u, rties)
            res = (res * QSCALE).astype(bf16)
            for j in range(2):
                QN[2 * u + j, pl.ds(TM * r, TM), :] = res[:, 128 * j:128 * (j + 1)]

        def vgemv(c0, dst, d0):
            acc = None
            marks = []
            for g in range(64):
                w = WMOD[16 * g:16 * g + 16, c0:c0 + 128].astype(f32) * SS[16 * g:16 * g + 16, :]
                t = w[0:8] + w[8:16]
                acc = t if acc is None else acc + t
                if g % 16 == 15:
                    marks.append(zero_of(acc))
            dst[:, d0:d0 + 128] = jnp.broadcast_to(jnp.sum(acc, axis=0, keepdims=True), (8, 128))
            return marks

        def sa_piece(i):
            m = jnp.dot(sc16, WMOD[:, 128 * i:128 * (i + 1)], preferred_element_type=f32)
            MOD1[:, 128 * i:128 * (i + 1)] = m[0:8]

        with scope('nat0'):
            with scope('w_x0'):
                cp_xn[0].wait()
            ln_nat(0)
            with scope('w_q0'):
                cp_w[0, 0].wait()
            qnat(0, 0, None)
            with scope('w_q1'):
                cp_w[0, 1].wait()
            qnat(0, 1, None)
            with scope('w_x1'):
                cp_xn[1].wait()
            ln_nat(1)

        def nat_region(waits, seq, extra=None, pre=None):
            for c_ in waits:
                c_.wait()
            T = Ties(['qkv'] * (2 * len(seq)))
            if pre:
                pre(T)
            for i, (r, ln_r) in enumerate(seq):
                if ln_r is not None:
                    T.spread(ln_nat(ln_r), 128 * i + nat_lo, 128 * i + nat_hi)
                for k, (rr, u) in enumerate(r):
                    qnat(rr, u, T.get(2 * i + k))
                    if extra:
                        extra(2 * i + k)

        with scope('nat1'):
            nat_region([cp_xn[2]], [([(1, 0), (1, 1)], 2)])
        with scope('nat2'):
            nat_region([cp_xn[3], cp_xn[4]], [([(2, 0), (2, 1)], 3), ([(3, 0), (3, 1)], 4)])
        with scope('nat3'):
            nat_region(cp_xn[5:], [([(4, 0), (4, 1)], 5), ([(5, 0), (5, 1)], 6)])
        with scope('nat4'):
            def sa_extra(d):
                for i in range(2 * d, 2 * d + 2):
                    sa_piece(i)
            def sa_vpu(T):
                T.spread([m_ for i in range(8) for m_ in vgemv(128 * i, MOD1, 128 * i)], 124, 250)
            if cfg.get('sa_vpu', 1):
                nat_region([cp_sa], [([(6, 0), (6, 1)], 7), ([(7, 0), (7, 1)], None)], None, sa_vpu)
            else:
                nat_region([cp_sa], [([(6, 0), (6, 1)], 7), ([(7, 0), (7, 1)], None)], sa_extra)

        for c_ in [cp_w[1, 0], cp_w[2, 0]]:
            c_.wait()
        sa_t = jnp.tile(MOD1[:, 0:1024], (128 // 8, 1))

        def make_hp(p):
            lo, hi = unpack2(load_words(HB, p))
            h = jnp.concatenate([lo + sa_t, hi + sa_t], axis=0).astype(bf16)
            HP[p] = h
            return h

        def bias_piece(i):
            sa16 = jnp.tile(MOD1[:, 0:1024], (2, 1)).astype(bf16)
            b = jnp.dot(sa16, WQKV[:, 128 * i:128 * (i + 1)], preferred_element_type=f32)[0:8] * QSCALE
            BQ[i] = jnp.tile(b, (16, 1)).T

        def rl_piece(u, j, p):
            w = QN.at[2 * u + j].bitcast(u32)[pl.ds(p, 128, stride=8), :]
            wt = w.T
            last = None
            for hf, val in enumerate(unpack2(wt)):
                val = val + BQ[2 * u + j]
                store_heads(Rset[u][0], 2 * p + hf, j, val)
                last = val
            return (pltpu.bitcast(last[120:128], u32) >> 31) >> 1

        with scope('kv0'):
            T = Ties(['qkv'] * 16)
            pieces = [(0, j, p) for p in range(NP) for j in range(2)]
            for p in range(NP):
                if p == 1:
                    T.spread([rl_piece(*pc) for pc in pieces], rl0_lo, rl0_hi)
                h = make_hp(p)
                for i, t in enumerate((1, 2)):
                    m, pns = qdot(h, WQKV, Rset[0][t], p, t, 0, T.get(2 * p + i))
                    if p == 0:
                        bias_piece(2 * i)
                        bias_piece(2 * i + 1)
                    for pn, sl in zip(pns, pin_sl):
                        T.add(64 * (2 * p + i + 1) + sl, pn)

        for c_ in [cp_w[1, 1], cp_w[2, 1], cp_wo]:
            c_.wait()
        with scope('unit1'):
            T = Ties(['qkv', 'qkv', 'out'] * NP)
            at = {}
            T.spread([rl_piece(1, j, p) for p in range(NP) for j in range(2)], rl1_lo, rl1_hi)
            for p in range(NP):
                for pp in (p, p + 1):
                    if pp < NP and pp not in at:
                        markers, words = attend_steps(RQ0, RK0, RV0, pp)
                        lo = max(192 * pp - u1_back, 8 if pp == 0 else 0)
                        T.spread(markers, lo, 192 * pp - u1_back + u1_len)
                        at[pp] = words
                h = HP[p]
                ms = []
                for i, t in enumerate((1, 2)):
                    m, pns = qdot(h, WQKV, Rset[1][t], p, t, 1, T.get(3 * p + i))
                    ms.append(m)
                    for pn, sl in zip(pns, pin_sl):
                        T.add(64 * (3 * p + i + 1) + sl, pn)
                store_o(OS0, p, at[p], zero_of(ms[1]))
                ACC[p] = out_dot(OS0, p, WO, 0, T.get(3 * p + 2))

        for c_ in [cp_w[t, u] for u in (2, 3) for t in range(3)] + [cp_mod2]:
            c_.wait()

        def gemv_piece(i):
            c0 = 128 * i
            g2 = jnp.dot(sc16, WMOD[:, pl.ds(2048 + c0, 128)], preferred_element_type=f32)
            MOD2[:, pl.ds(c0, 128)] = g2[0:8, :]

        seq = []
        for p in range(NP):
            seq += [('q', 2, 0, p), ('q', 2, 1, p), ('q', 2, 2, p), ('o', 1, p)]
        for p in range(NP):
            seq += [('q', 3, 1, p), ('q', 3, 2, p)]
        seq += [('q', 3, 0, p) for p in range(NP)] + [('o', 2, p) for p in range(NP)] + [('o', 3, p) for p in range(NP)]
        T = Ties(['qkv' if op[0] == 'q' else 'out' for op in seq])
        wins = [(1, p, a1_lo + p * a1_w, a1_lo + p * a1_w + a1_len) for p in range(NP)]
        wins += [(2, p, a2_lo + p * a2_w, a2_lo + p * a2_w + a2_len) for p in range(NP)]
        wins += [(3, p, a3_lo + p * a3_w, a3_lo + p * a3_w + a3_len) for p in range(NP)]
        pend = {}
        with scope('u23t'):
            for d, op in enumerate(seq):
                for (ua, p, lo, hi) in wins:
                    if (ua, p) not in pend and lo // 64 <= d:
                        Ra = Rset[ua % 2]
                        markers, words = attend_steps(Ra[0], Ra[1], Ra[2], p)
                        T.spread(markers, lo, hi)
                        pend[(ua, p)] = words
                if op[0] == 'q':
                    _, u, t, p = op
                    m, pns = qdot(HP[p], WQKV, Rset[u % 2][t], p, t, u, T.get(d))
                    for pn, sl in zip(pns, pin_sl):
                        T.add(64 * (d + 1) + sl, pn)
                else:
                    _, u, p = op
                    assert pend.get((u, p), 0) is None, (u, p)
                    res = out_dot(OSs[u % 2], p, WO, u, T.get(d))
                    m = res[0:8, 0:128]
                if g_mode == 'mxu':
                    if d < 32:
                        gemv_piece(d)
                elif g_lo <= d + 1 < g_lo + 32:
                    gi = d + 1 - g_lo
                    T.spread(vgemv(2048 + 128 * gi, MOD2, 128 * gi), 64 * (d + 1) + 6, 64 * (d + 1) + 64)
                for (ua, pp, lo, hi) in wins:
                    if pend.get((ua, pp)) is not None and (hi + thr) // 64 <= d:
                        store_o(OSs[ua % 2], pp, pend[(ua, pp)], zero_of(m))
                        pend[(ua, pp)] = None
                if op[0] == 'o':
                    if u < 3:
                        ACC[p] += res
                    else:
                        ga_t = jnp.tile(MOD2[:, 0:1024], (128 // 8, 1))
                        a = ACC[p] + res
                        x1w = pack2(ga_t * a[0:128], ga_t * a[128:256])
                        for j in range(8):
                            X1B[j, pl.ds(p, 128, stride=8), :] = x1w[:, 128 * j:128 * (j + 1)]

        TC = 256

        def x1_rows(r0w):
            br = jnp.concatenate([pltpu.bitcast(X1B[j, pl.ds(r0w, 64), :], bf16) for j in range(8)], axis=1)
            r0 = 2 * r0w if isinstance(r0w, int) else pl.multiple_of(2 * r0w, 128)
            return (XN[pl.ds(r0, 128), :].astype(f32) + br.astype(f32)).astype(bf16).astype(f32)

        def ln2_rows(r0w):
            b1 = jnp.tile(1.0 + MOD2[:, 2048:3072], (128 // 8, 1))
            sb = jnp.tile(MOD2[:, 1024:2048], (128 // 8, 1))
            return layer_norm(x1_rows(r0w)) * b1 + sb

        def epilogue(rp, k, rdst):
            w0 = pl.multiple_of(rp * 128 + k * 64, 64)
            gbt = jnp.tile(MOD2[:, 3072:4096], (128 // 8, 1))
            a0 = pl.multiple_of(k * 128, 128)
            out = x1_rows(w0) + gbt * ACC[rp % 2, pl.ds(a0, 128), :]
            r0 = pl.multiple_of(rdst * 256 + k * 128, 128)
            OUTB[pl.ds(r0, 128), :] = out.astype(bf16)
            return out

        def out_copy(i):
            r0 = i * 128 if isinstance(i, int) else pl.multiple_of(i * 128, 128)
            return pltpu.make_async_copy(OUTB.at[pl.ds(r0, 128), :], out_hbm.at[0, pl.ds(r0, 128), :],
                                         sems.at[sem_i[0] + i])

        def pins_of(v):
            b = pltpu.bitcast(v, u32)
            return [(or_all([b[16 * g + 8 * i:16 * g + 8 * i + 8, 128 * j:128 * (j + 1)]
                             for i in range(2) for j in range(8)]) >> 31) >> 1 for g in range(8)]

        with scope('ln2_0'):
            H2T[0, 0:128, :] = ln2_rows(0).astype(bf16)
            H2T[0, 128:256, :] = ln2_rows(64).astype(bf16)
        for c_ in cp_ffn:
            c_.wait()

        def ffn_body(i, _):
            r = i // 2
            k = i % 2
            h = H2T[r % 2]
            hn = ln2_rows(pl.multiple_of(jnp.minimum(r + 1, 7) * 128 + k * 64, 64))
            H2T[(r + 1) % 2, pl.ds(pl.multiple_of(k * 128, 128), 128), :] = hn.astype(bf16)
            pa = pins_of(hn)
            pb = pins_of(epilogue(jnp.maximum(r - 1, 0), k, jnp.where(r == 0, 8, r - 1)))
            acc = None
            for j in range(TH // TC):
                sel = {}
                for g in range(8):
                    if 1 + g // 2 == j:
                        sel[(4 * (g % 2), 0)] = pa[g]
                    if 2 + g // 2 == j:
                        sel[(4 * (g % 2) + 8, 0)] = pb[g]
                cs = pl.ds(j * TC, TC)
                g_ = jnp.dot(tie_lhs(h, sel), W1[k, :, cs], preferred_element_type=f32)
                up = jnp.dot(h, W3[k, :, cs], preferred_element_type=f32)
                a = (g_ * jax.nn.sigmoid(g_) * up).astype(bf16)
                o = jnp.dot(a, W2[k, cs, :], preferred_element_type=f32)
                acc = o if acc is None else acc + o
            ACC[r % 2] = acc + jnp.where(k == 0, 0.0, ACC[r % 2])

            @pl.when(i >= 2)
            def _():
                out_copy(i - 2).start()
            return 0
        with scope('ffn'):
            lax.fori_loop(0, 16, ffn_body, 0)
        with scope('tail'):
            epilogue(7, 0, 7)
            out_copy(14).start()
            epilogue(7, 1, 7)
            out_copy(15).start()
            for i in range(16):
                out_copy(i).wait()

    return kernel


def build(cfg=None):
    cfg = cfg or {}
    kernel = make_kernel(cfg)
    V = pltpu.VMEM
    scratch = [
        V((1, D), bf16),
        V((D, 128), f32),
        V((8, SPAD, 128), bf16),
        V((4, SPAD, 128), bf16),
        V((4, 128, 128), f32),
        V((NP, TM, D), bf16),
        V((D, 3 * D), bf16),
        V((16, 264, 128), f32), V((32, 264, 128), f32), V((32, 264, 128), f32),
        V((16, 264, 128), f32), V((32, 264, 128), f32), V((32, 264, 128), f32),
        V((NP, 272, 128), u32), V((NP, 272, 128), u32),
        V((D, D), bf16),
        V((NP, TM, D), f32),
        V((2, TM, D), bf16),
        V((8, WPAD, 128), u32),
        V((2, D, F // 2), bf16), V((2, D, F // 2), bf16), V((2, F // 2, D), bf16),
        V((D, 6 * D), bf16),
        V((S + TM, D), bf16),
        V((8, 2 * D), f32),
        V((8, 4 * D), f32),
        pltpu.SemaphoreType.DMA((64,)),
    ]
    anyspec = pl.BlockSpec(memory_space=pl.ANY)
    return pl.pallas_call(
        kernel,
        out_shape=jax.ShapeDtypeStruct((1, S, D), bf16),
        in_specs=[anyspec] * 8,
        out_specs=anyspec,
        scratch_shapes=scratch,
        compiler_params=pltpu.CompilerParams(vmem_limit_bytes=cfg.get('vmem', 124 * 2 ** 20), flags=cfg.get('flags')),
    )


@jax.jit
def pallas_adaLN_cond__sliding_local_dilated__glu_gated_swiglu__prompt_kernel(
    A_x: jax.Array,
    A_wqkv: jax.Array,
    A_wo: jax.Array,
    B_x: jax.Array,
    B_w1: jax.Array,
    B_w3: jax.Array,
    B_w2: jax.Array,
    c: jax.Array,
    w_mod: jax.Array,
):
    del B_x
    return build({})(A_x, A_wqkv, A_wo, B_w1, B_w3, B_w2, c, w_mod)
```
